```python
import os as _os
_os.environ.setdefault("JAX_PLATFORMS", "cpu")
import jax
import jax.numpy as jnp

def _softmax(x, axis=-1):
    return jax.nn.softmax(x, axis=axis)
def _gelu(x):
    return jax.nn.gelu(x, approximate=True)
def _silu(x):
    return jax.nn.silu(x)
def _sigmoid(x):
    return jax.nn.sigmoid(x)
def _layernorm(x, axis=-1, eps=1e-5):
    m = jnp.mean(x, axis=axis, keepdims=True)
    v = jnp.var(x, axis=axis, keepdims=True)
    return (x - m) / jnp.sqrt(v + eps)
def _scatter_add(tgt, idx, src, axis=0):
    return tgt.at[idx].add(src)
def _segment_sum(src, seg, n):
    return jax.ops.segment_sum(src, seg, n)
class _Rng:
    def __init__(self, key):
        self._k = key
    def _next(self):
        self._k, sub = jax.random.split(self._k)
        return sub
    def normal(self, shape):
        return jax.random.normal(self._next(), shape, dtype=jnp.bfloat16)
    def randint(self, lo, hi, shape):
        return jax.random.randint(self._next(), shape, lo, hi, dtype=jnp.int32)
    def uniform(self, shape, lo=0.0, hi=1.0):
        return jax.random.uniform(self._next(), shape, jnp.bfloat16, lo, hi)
    def permutation(self, n):
        return jax.random.permutation(self._next(), n)


kernel_name = 'concat_heads__mha_block_cached__gqa_block_cached__near_ridge'

def setup_inputs():
    _rng = _Rng(jax.random.key(int.from_bytes(__import__("os").urandom(4), "little")))
    _w = (lambda a: (lambda t: t.astype(jnp.bfloat16) if jnp.issubdtype(t.dtype, jnp.floating) else t)(jnp.asarray(a)))
    def _A_setup():
        B, Sq, D = 8, 128, 640
        H, Sk, Dh = 32, 1024, 192
        return {
            "x": _w((lambda *s: _rng.normal(s) * 0.8)(B, Sq, D)),
            "k_cache": _w((lambda *s: _rng.normal(s) * 0.8)(B, H, Sk, Dh)),
            "v_cache": _w((lambda *s: _rng.normal(s) * 0.05)(B, H, Sk, Dh)),
            "wq": _w((lambda *s: _rng.normal(s) * 0.8)(D, H * Dh) * (D ** -0.5)),
            "wo": _w((lambda *s: _rng.normal(s) * 0.05)(H * Dh, D) * ((H * Dh) ** -0.5)),
        }
    _A_in = _A_setup()

    def _B_setup():
        B, Sq, D = 8, 128, 640
        Hq, Hkv, Sk, Dh = 32, 32, 1024, 192
        assert Hq % Hkv == 0, (Hq, Hkv)
        return {
            "x": _w((lambda *s: _rng.normal(s) * 0.8)(B, Sq, D)),
            "k_cache": _w((lambda *s: _rng.normal(s) * 0.8)(B, Hkv, Sk, Dh)),
            "v_cache": _w((lambda *s: _rng.normal(s) * 0.05)(B, Hkv, Sk, Dh)),
            "wq": _w((lambda *s: _rng.normal(s) * 0.8)(D, Hq * Dh) * (D ** -0.5)),
            "wo": _w((lambda *s: _rng.normal(s) * 0.05)(Hq * Dh, D) * ((Hq * Dh) ** -0.5)),
        }
    _B_in = _B_setup()

    return {
        "A_x": _A_in["x"],
        "A_k_cache": _A_in["k_cache"],
        "A_v_cache": _A_in["v_cache"],
        "A_wq": _A_in["wq"],
        "A_wo": _A_in["wo"],
        "B_x": _B_in["x"],
        "B_k_cache": _B_in["k_cache"],
        "B_v_cache": _B_in["v_cache"],
        "B_wq": _B_in["wq"],
        "B_wo": _B_in["wo"],
    }

def reference(A_x, A_k_cache, A_v_cache, A_wq, A_wo, B_x, B_k_cache, B_v_cache, B_wq, B_wo):
    def _A_ref(x, k_cache, v_cache, wq, wo):
        B, Sq, D = x.shape
        H, Dh = 32, 192
        q = (lambda x, *d: x.transpose(*d))((x @ wq).reshape(B, Sq, H, Dh), 0, 2, 1, 3)
        scores = jnp.einsum("bhqd,bhkd->bhqk", q, k_cache) * (Dh ** -0.5)
        p = _softmax(scores, axis=-1)
        o = jnp.einsum("bhqk,bhkd->bhqd", p, v_cache)
        return (lambda x, *d: x.transpose(*d))(o, 0, 2, 1, 3).reshape(B, Sq, H * Dh) @ wo

    def _B_ref(x, k_cache, v_cache, wq, wo):
        B, Sq, D = x.shape
        Hq, Dh = 32, 192
        Hkv = k_cache.shape[1]
        rep = Hq // Hkv
        q = (lambda x, *d: x.transpose(*d))((x @ wq).reshape(B, Sq, Hq, Dh), 0, 2, 1, 3)
        k = jnp.repeat(k_cache, rep, axis=1)
        v = jnp.repeat(v_cache, rep, axis=1)
        scores = jnp.einsum("bhqd,bhkd->bhqk", q, k) * (Dh ** -0.5)
        p = _softmax(scores, axis=-1)
        o = jnp.einsum("bhqk,bhkd->bhqd", p, v)
        return (lambda x, *d: x.transpose(*d))(o, 0, 2, 1, 3).reshape(B, Sq, Hq * Dh) @ wo

    a = _A_ref(A_x, A_k_cache, A_v_cache, A_wq, A_wo)
    b = _B_ref(B_x, B_k_cache, B_v_cache, B_wq, B_wo)
    return jnp.concatenate([a, b], axis=-1)
```

```python
import functools
import math
import jax
import jax.numpy as jnp
from jax import lax
import jax.experimental.pallas as pl
import jax.experimental.pallas.tpu as pltpu

B, SQ, D = 8, 128, 640
H, SK, DH = 32, 1024, 192
PAIR = 2 * DH
NHP = H // 2
NG = 2 * NHP
NU = NG * B
QSCALE = (DH ** -0.5) * math.log2(math.e)
NBUF = 8
NW = 4
COMPUTE = True
F32 = jnp.float32
BF16 = jnp.bfloat16


def _kernel(xa, ka, va, wqa, woa, xb, kb, vb, wqb, wob, out_hbm,
            kbuf, vbuf, wqbuf, wobuf, xbuf, acc, obuf, qbuf, otbuf, invbuf,
            ksem, vsem, wqsem, wosem, xsem, osem):

    def kv_copies(br, n):
        g = n // B
        b = n % B
        p = g % NHP
        slot = n % NBUF
        k_hbm, v_hbm = (ka, va) if br == 0 else (kb, vb)
        return (pltpu.make_async_copy(k_hbm.at[b, p], kbuf.at[slot], ksem.at[slot]),
                pltpu.make_async_copy(v_hbm.at[b, p], vbuf.at[slot], vsem.at[slot]))

    def wq_copy(br, g):
        p = g % NHP
        w = wqa if br == 0 else wqb
        c0 = p * PAIR if isinstance(p, int) else pl.multiple_of(p * PAIR, 128)
        return pltpu.make_async_copy(w.at[:, pl.ds(c0, PAIR)], wqbuf.at[g % NW], wqsem.at[g % NW])

    def wo_copy(br, g):
        p = g % NHP
        w = woa if br == 0 else wob
        r0 = p * PAIR if isinstance(p, int) else pl.multiple_of(p * PAIR, 128)
        return pltpu.make_async_copy(w.at[pl.ds(r0, PAIR), :], wobuf.at[g % NW], wosem.at[g % NW])

    def x_copy(br):
        return pltpu.make_async_copy(xa if br == 0 else xb, xbuf.at[br], xsem.at[br])

    def out_copy(br, b):
        r0 = b * SQ if isinstance(b, int) else pl.multiple_of(b * SQ, SQ)
        return pltpu.make_async_copy(obuf.at[br, pl.ds(r0, SQ), :],
                                     out_hbm.at[pl.ds(r0, SQ), br * D:(br + 1) * D],
                                     osem.at[br * B + b])

    def issue_unit(br, n):
        kc, vc = kv_copies(br, n)
        kc.start()
        vc.start()

    x_copy(0).start()
    wq_copy(0, 0).start()
    issue_unit(0, 0)
    wo_copy(0, 0).start()
    for n in range(1, NBUF - 1):
        if (n + 1) % B == 0:
            wq_copy(0, (n + 1) // B).start()
        issue_unit(0, n)
        if n % B == 0:
            wo_copy(0, n // B).start()
    x_copy(1).start()

    acc[...] = jnp.zeros(acc.shape, F32)
    otbuf[...] = jnp.zeros(otbuf.shape, F32)
    invbuf[...] = jnp.zeros(invbuf.shape, F32)

    lane = lax.broadcasted_iota(jnp.int32, (SQ, 128), 1)

    def qproj(n):
        g = n // B
        b = n % B
        br = g // NHP
        r0 = pl.multiple_of(b * SQ, SQ)
        q = jnp.dot(xbuf[br, pl.ds(r0, SQ), :], wqbuf[g % NW], preferred_element_type=F32) * QSCALE
        qb = q[:, 128:256]
        qq = jnp.concatenate([q[:, 0:128], jnp.where(lane < 64, qb, 0.0),
                              jnp.where(lane >= 64, qb, 0.0), q[:, 256:384]], axis=1)
        qbuf[n % 2] = qq.astype(BF16)

    def oproj(n):
        g = n // B
        b = n % B
        br = g // NHP
        r0 = pl.multiple_of(b * SQ, SQ)
        o = otbuf[...].T * invbuf[...]
        acc[br, pl.ds(r0, SQ), :] += jnp.dot(o.astype(BF16), wobuf[g % NW], preferred_element_type=F32)

    x_copy(0).wait()
    wq_copy(0, 0).wait()
    wo_copy(0, 0).wait()
    if COMPUTE:
        qproj(0)

    def body(u, carry):
        n = u - 1 + NBUF
        for br in range(2):
            lo, hi = br * (NU // 2), (br + 1) * (NU // 2)

            @pl.when(jnp.logical_and(n + 1 >= lo, jnp.logical_and(n + 1 < hi, (n + 1) % B == 0)))
            def _():
                wq_copy(br, (n + 1) // B).start()

            @pl.when(jnp.logical_and(n >= lo, n < hi))
            def _():
                issue_unit(br, n)

            @pl.when(jnp.logical_and(n >= lo, jnp.logical_and(n < hi, n % B == 0)))
            def _():
                wo_copy(br, n // B).start()

        kc, vc = kv_copies(0, u)
        kc.wait()
        vc.wait()

        @pl.when(jnp.logical_and((u + 1) % B == 0, u + 1 < NU))
        def _():
            wq_copy(0, (u + 1) // B).wait()

        @pl.when(jnp.logical_and((u - 1) % B == 0, u > B))
        def _():
            wo_copy(0, (u - 1) // B).wait()

        @pl.when(u == NU // 2 - 1)
        def _():
            x_copy(1).wait()

        if COMPUTE:
            slot = u % NBUF
            kt = kbuf.at[slot]
            vt = vbuf.at[slot]
            qq = qbuf[u % 2]
            s1 = jnp.dot(qq[:, 0:256], kt[0:256, :], preferred_element_type=F32)
            s2 = jnp.dot(qq[:, 256:512], kt[128:384, :], preferred_element_type=F32)
            oproj(jnp.maximum(u - 1, 0))
            m1 = jnp.max(s1, axis=-1, keepdims=True)
            p1 = jnp.exp2(s1 - m1)
            l1 = jnp.sum(p1, axis=-1, keepdims=True)
            ot1 = lax.dot_general(vt[0:DH, :], p1.astype(BF16), (((1,), (1,)), ((), ())),
                                  preferred_element_type=F32)
            qproj(jnp.minimum(u + 1, NU - 1) )
            m2 = jnp.max(s2, axis=-1, keepdims=True)
            p2 = jnp.exp2(s2 - m2)
            l2 = jnp.sum(p2, axis=-1, keepdims=True)
            ot2 = lax.dot_general(vt[DH:PAIR, :], p2.astype(BF16), (((1,), (1,)), ((), ())),
                                  preferred_element_type=F32)
            otbuf[0:DH, :] = ot1
            otbuf[DH:PAIR, :] = ot2
            i1 = jnp.broadcast_to(1.0 / l1, (SQ, 128))
            i2 = jnp.broadcast_to(1.0 / l2, (SQ, 128))
            invbuf[...] = jnp.concatenate([i1, jnp.where(lane < 64, i1, i2), i2], axis=1)

        w = u - 1
        for br in range(2):
            @pl.when(w // B == br * NHP + NHP - 1)
            def _():
                b = w % B
                r0 = pl.multiple_of(b * SQ, SQ)
                obuf[br, pl.ds(r0, SQ), :] = acc[br, pl.ds(r0, SQ), :].astype(BF16)
                out_copy(br, b).start()
        return carry

    lax.fori_loop(0, NU, body, 0)

    if COMPUTE:
        oproj(NU - 1)
    obuf[1, (B - 1) * SQ:B * SQ, :] = acc[1, (B - 1) * SQ:B * SQ, :].astype(BF16)
    out_copy(1, B - 1).start()
    for br in range(2):
        for b in range(B):
            out_copy(br, b).wait()


@jax.jit
def pallas_concat_heads__mha_block_cached__gqa_block_cached__near_ridge_kernel(
    A_x, A_k_cache, A_v_cache, A_wq, A_wo, B_x, B_k_cache, B_v_cache, B_wq, B_wo,
):
    def kv(a):
        return jnp.swapaxes(a, 2, 3).reshape(B, NHP, PAIR, SK)

    any_spec = pl.BlockSpec(memory_space=pl.ANY)
    out = pl.pallas_call(
        _kernel,
        in_specs=[any_spec] * 10,
        out_specs=any_spec,
        out_shape=jax.ShapeDtypeStruct((B * SQ, 2 * D), BF16),
        scratch_shapes=[
            pltpu.VMEM((NBUF, PAIR, SK), BF16),
            pltpu.VMEM((NBUF, PAIR, SK), BF16),
            pltpu.VMEM((NW, D, PAIR), BF16),
            pltpu.VMEM((NW, PAIR, D), BF16),
            pltpu.VMEM((2, B * SQ, D), BF16),
            pltpu.VMEM((2, B * SQ, D), F32),
            pltpu.VMEM((2, B * SQ, D), BF16),
            pltpu.VMEM((2, SQ, 512), BF16),
            pltpu.VMEM((PAIR, SQ), F32),
            pltpu.VMEM((SQ, PAIR), F32),
            pltpu.SemaphoreType.DMA((NBUF,)),
            pltpu.SemaphoreType.DMA((NBUF,)),
            pltpu.SemaphoreType.DMA((NW,)),
            pltpu.SemaphoreType.DMA((NW,)),
            pltpu.SemaphoreType.DMA((2,)),
            pltpu.SemaphoreType.DMA((2 * B,)),
        ],
        compiler_params=pltpu.CompilerParams(
            vmem_limit_bytes=100 * 1024 * 1024,
        ),
    )(A_x.reshape(B * SQ, D), kv(A_k_cache), kv(A_v_cache), A_wq, A_wo,
      B_x.reshape(B * SQ, D), kv(B_k_cache), kv(B_v_cache), B_wq, B_wo)
    return out.reshape(B, SQ, 2 * D)
```

```python
import math
import jax
import jax.numpy as jnp
from jax import lax
import jax.experimental.pallas as pl
import jax.experimental.pallas.tpu as pltpu

B, SQ, D = 8, 128, 640
H, SK, DH = 32, 1024, 192
PAIR = 2 * DH
NHP = H // 2
NI = NHP * B
QSCALE = (DH ** -0.5) * math.log2(math.e)
NBUF = 4
NW = 4
KCH = 16
NSTEP = DH // KCH
PH = 9
WLEAD = 2
COMPUTE = True
F32 = jnp.float32
BF16 = jnp.bfloat16
NT = (((1,), (1,)), ((), ()))


def _mo(x, m):
    return x if isinstance(x, int) else pl.multiple_of(x, m)


def _when(cond, fn):
    if isinstance(cond, bool):
        if cond:
            fn()
    else:
        pl.when(cond)(fn)


def _kernel(xa, ka, va, wqa, woa, xb, kb, vb, wqb, wob, out_hbm,
            kvbuf, wqbuf, wobuf, xbuf, acc, obuf, qbuf, otbuf, invbuf,
            kvsem, wqsem, wosem, xsem, osem):

    def issue_step(i, t):
        vi = i + (t + PH) // NSTEP
        j = (t + PH) % NSTEP
        for lag in range(2):
            n = vi + 2 - lag
            valid = (0 <= n < NI) if isinstance(n, int) else (n < NI)

            def go(n=n, lag=lag):
                slot = n & (NBUF - 1)
                b = n & 7
                p = (n >> 3) & (NHP - 1)
                r0 = lag * DH + j * KCH
                for br in range(2):
                    for kv in range(2):
                        src = ((ka, va), (kb, vb))[br][kv]
                        pltpu.make_async_copy(src.at[b, p, pl.ds(r0, KCH), :],
                                              kvbuf.at[slot, br, kv, pl.ds(r0, KCH), :],
                                              kvsem.at[slot]).start(priority=kv)
            _when(valid, go)

    def wait_slot(buf, sem, slot):
        pltpu.make_async_copy(buf.at[slot], buf.at[slot], sem.at[slot]).wait()

    def issue_w(g, j):
        p = g & (NHP - 1)
        slot = g & (NW - 1)
        c0 = _mo(p * PAIR, 128)
        for h in range(2):
            for br, w in enumerate((wqa, wqb)):
                r0 = _mo(j * 80 + h * 40, 8)
                pltpu.make_async_copy(w.at[pl.ds(r0, 40), pl.ds(c0, PAIR)],
                                      wqbuf.at[slot, br, pl.ds(r0, 40), :], wqsem.at[slot]).start(priority=0)
        for h in range(2):
            for br, w in enumerate((woa, wob)):
                r0 = _mo(j * 48 + h * 24, 8)
                pltpu.make_async_copy(w.at[pl.ds(_mo(p * PAIR + r0, 8), 24), :],
                                      wobuf.at[slot, br, pl.ds(r0, 24), :], wosem.at[slot]).start(priority=1)

    def out_copy(b):
        r0 = _mo(b * SQ, SQ)
        return pltpu.make_async_copy(obuf.at[pl.ds(r0, SQ), :], out_hbm.at[pl.ds(r0, SQ), :], osem.at[b])

    for c in range(B * SQ // 32):
        for br, src in enumerate((xa, xb)):
            pltpu.make_async_copy(src.at[pl.ds(c * 32, 32), :], xbuf.at[0, br, pl.ds(c * 32, 32), :],
                                  xsem.at[0]).start(priority=br)
    for j in range(B):
        issue_w(0, j)
    for j in range(WLEAD):
        issue_w(1, j)
    for i in range(-4, 0):
        for t in range(NSTEP):
            issue_step(i, t)

    acc[...] = jnp.zeros(acc.shape, F32)
    otbuf[...] = jnp.zeros(otbuf.shape, F32)
    invbuf[...] = jnp.zeros(invbuf.shape, F32)

    lane = lax.broadcasted_iota(jnp.int32, (SQ, 128), 1)

    def qproj(br, n):
        r0 = _mo((n & 7) * SQ, SQ)
        q = jnp.dot(xbuf[0, br, pl.ds(r0, SQ), :], wqbuf[(n >> 3) & (NW - 1), br],
                    preferred_element_type=F32) * QSCALE
        qb = q[:, 128:256]
        qq = jnp.concatenate([q[:, 0:128], jnp.where(lane < 64, qb, 0.0),
                              jnp.where(lane >= 64, qb, 0.0), q[:, 256:384]], axis=1)
        return qq.astype(BF16)

    def oproj(br, n, ot, inv):
        r0 = _mo((n & 7) * SQ, SQ)
        o = ot.T * inv
        acc[pl.ds(r0, SQ), br * D:(br + 1) * D] += jnp.dot(
            o.astype(BF16), wobuf[(n >> 3) & (NW - 1), br], preferred_element_type=F32)

    def qk(qq, kt, hook):
        parts = []
        for h in range(2):
            for c in range(2):
                if COMPUTE:
                    parts.append(jnp.dot(qq[:, h * 256:(h + 1) * 256],
                                         kt[h * 128:h * 128 + 256, c * 512:(c + 1) * 512],
                                         preferred_element_type=F32))
                hook()
        if COMPUTE:
            return jnp.concatenate(parts[0:2], axis=1), jnp.concatenate(parts[2:4], axis=1)
        return None, None

    def softmax_pv(s, v):
        m = jnp.max(s, axis=-1, keepdims=True)
        p = jnp.exp2(s - m)
        l = jnp.sum(p, axis=-1, keepdims=True)
        ot = lax.dot_general(v, p.astype(BF16), NT, preferred_element_type=F32)
        return ot, jnp.broadcast_to(1.0 / l, (SQ, 128))

    def mk_inv(i1, i2):
        return jnp.concatenate([i1, jnp.where(lane < 64, i1, i2), i2], axis=1)

    wait_slot(xbuf, xsem, 0)
    wait_slot(wqbuf, wqsem, 0)
    wait_slot(wobuf, wosem, 0)
    if COMPUTE:
        qbuf[...] = qproj(0, 0)

    def body(i, carry):
        slot = i & (NBUF - 1)
        wait_slot(kvbuf, kvsem, slot)

        @pl.when(jnp.logical_and((i & 7) == 7, i < NI - 1))
        def _():
            wait_slot(wqbuf, wqsem, ((i + 1) >> 3) & (NW - 1))

        @pl.when(jnp.logical_and((i & 7) == 0, i > 0))
        def _():
            wait_slot(wobuf, wosem, (i >> 3) & (NW - 1))

        n0 = i + WLEAD
        gw = (n0 >> 3) + 1

        @pl.when(gw < NHP)
        def _():
            issue_w(gw, n0 & 7)

        step = [0]

        def hook():
            issue_step(i, step[0])
            step[0] += 1

        sa1, sa2 = qk(qbuf[...], kvbuf.at[slot, 0, 0], hook)
        if COMPUTE:
            oproj(1, jnp.maximum(i - 1, 0), otbuf[...], invbuf[...])
            ota1, ia1 = softmax_pv(sa1, kvbuf[slot, 0, 1, 0:DH, :])
        hook()
        if COMPUTE:
            qqb = qproj(1, i)
            ota2, ia2 = softmax_pv(sa2, kvbuf[slot, 0, 1, DH:PAIR, :])
        else:
            qqb = None
        hook()
        sb1, sb2 = qk(qqb, kvbuf.at[slot, 1, 0], hook)
        if COMPUTE:
            oproj(0, i, jnp.concatenate([ota1, ota2], axis=0), mk_inv(ia1, ia2))
            otb1, ib1 = softmax_pv(sb1, kvbuf[slot, 1, 1, 0:DH, :])
        hook()
        if COMPUTE:
            qbuf[...] = qproj(0, jnp.minimum(i + 1, NI - 1))
            otb2, ib2 = softmax_pv(sb2, kvbuf[slot, 1, 1, DH:PAIR, :])
        hook()
        if COMPUTE:
            otbuf[0:DH, :] = otb1
            otbuf[DH:PAIR, :] = otb2
            invbuf[...] = mk_inv(ib1, ib2)
        assert step[0] == NSTEP

        @pl.when(i > NI - B)
        def _():
            b = (i - 1) & 7
            r0 = pl.multiple_of(b * SQ, SQ)
            obuf[pl.ds(r0, SQ), :] = acc[pl.ds(r0, SQ), :].astype(BF16)
            out_copy(b).start()
        return carry

    lax.fori_loop(0, NI, body, 0)

    if COMPUTE:
        oproj(1, NI - 1, otbuf[...], invbuf[...])
    obuf[(B - 1) * SQ:B * SQ, :] = acc[(B - 1) * SQ:B * SQ, :].astype(BF16)
    out_copy(B - 1).start()
    for b in range(B):
        out_copy(b).wait()


@jax.jit
def pallas_concat_heads__mha_block_cached__gqa_block_cached__near_ridge_kernel(
    A_x, A_k_cache, A_v_cache, A_wq, A_wo, B_x, B_k_cache, B_v_cache, B_wq, B_wo,
):
    def kv(a):
        return jnp.swapaxes(a, 2, 3).reshape(B, NHP, PAIR, SK)

    any_spec = pl.BlockSpec(memory_space=pl.ANY)
    out = pl.pallas_call(
        _kernel,
        in_specs=[any_spec] * 10,
        out_specs=any_spec,
        out_shape=jax.ShapeDtypeStruct((B * SQ, 2 * D), BF16),
        scratch_shapes=[
            pltpu.VMEM((NBUF, 2, 2, PAIR, SK), BF16),
            pltpu.VMEM((NW, 2, D, PAIR), BF16),
            pltpu.VMEM((NW, 2, PAIR, D), BF16),
            pltpu.VMEM((1, 2, B * SQ, D), BF16),
            pltpu.VMEM((B * SQ, 2 * D), F32),
            pltpu.VMEM((B * SQ, 2 * D), BF16),
            pltpu.VMEM((SQ, 512), BF16),
            pltpu.VMEM((PAIR, SQ), F32),
            pltpu.VMEM((SQ, PAIR), F32),
            pltpu.SemaphoreType.DMA((NBUF,)),
            pltpu.SemaphoreType.DMA((NW,)),
            pltpu.SemaphoreType.DMA((NW,)),
            pltpu.SemaphoreType.DMA((1,)),
            pltpu.SemaphoreType.DMA((B,)),
        ],
        compiler_params=pltpu.CompilerParams(
            vmem_limit_bytes=100 * 1024 * 1024,
        ),
    )(A_x.reshape(B * SQ, D), kv(A_k_cache), kv(A_v_cache), A_wq, A_wo,
      B_x.reshape(B * SQ, D), kv(B_k_cache), kv(B_v_cache), B_wq, B_wo)
    return out.reshape(B, SQ, 2 * D)
```

```python
import math
import jax
import jax.numpy as jnp
from jax import lax
import jax.experimental.pallas as pl
import jax.experimental.pallas.tpu as pltpu

B, SQ, D = 8, 128, 640
H, SK, DH = 32, 1024, 192
PAIR = 2 * DH
NHP = H // 2
NI = NHP * B
QSCALE = (DH ** -0.5) * math.log2(math.e)
NBUF = 4
NW = 4
KCH = 16
NSTEP = DH // KCH
PH = 4
WLEAD = 2
SH = 13
ROT = (0, 0, 6)
OUT_AT = 126
COMPUTE = True
F32 = jnp.float32
BF16 = jnp.bfloat16
NT = (((1,), (1,)), ((), ()))


NTILE = PAIR
WIDE = NTILE * 128
VISITS = [[(t0, t1) for t0, t1 in ((NTILE - 16 + SH, NTILE), (0, SH)) if t1 > t0]] + [
    [(SH + 16 * k, SH + 16 * (k + 1))] for k in range(NTILE // 16 - 1)]


def _mo(x, m):
    return x if isinstance(x, int) else pl.multiple_of(x, m)


def _when(cond, fn):
    if isinstance(cond, bool):
        if cond:
            fn()
    else:
        pl.when(cond)(fn)


def _kernel(xa, ka, va, wqa, woa, xb, kb, vb, wqb, wob, out_hbm,
            kvbuf, wqbuf, wobuf, xbuf, acc, obuf, qbuf, otbuf, invbuf,
            kvsem, wqsem, wosem, xsem, osem):

    def issue_step(i, t):
        vi = i + (t + PH) // NSTEP
        j = (t + PH) % NSTEP
        for br in range(2):
            for kv in range(2):
                for lag in (1, 0):
                    n = vi + 2 - lag
                    valid = (0 <= n < NI) if isinstance(n, int) else (n < NI)

                    def go(n=n, lag=lag, br=br, kv=kv):
                        slot = n & (NBUF - 1)
                        b = n & 7
                        p = (n >> 3) & (NHP - 1)
                        k = lag * NSTEP + (j + ROT[0] * kv + ROT[1] * br + ROT[2] * lag) % NSTEP
                        src = ((ka, va), (kb, vb))[br][kv]
                        for t0, t1 in VISITS[k]:
                            cols = pl.ds(t0 * 128, (t1 - t0) * 128)
                            pltpu.make_async_copy(src.at[b, p, :, cols],
                                                  kvbuf.at[slot, br, kv, :, cols],
                                                  kvsem.at[slot]).start(priority=1 - lag)
                    _when(valid, go)

    def wait_slot(buf, sem, slot):
        pltpu.make_async_copy(buf.at[slot], buf.at[slot], sem.at[slot]).wait()

    def issue_w(g, j):
        p = g & (NHP - 1)
        slot = g & (NW - 1)
        c0 = _mo(p * PAIR, 128)
        for h in range(2):
            for br, w in enumerate((wqa, wqb)):
                r0 = _mo(j * 80 + h * 40, 8)
                pltpu.make_async_copy(w.at[pl.ds(r0, 40), pl.ds(c0, PAIR)],
                                      wqbuf.at[slot, br, pl.ds(r0, 40), :], wqsem.at[slot]).start(priority=0)
        for h in range(2):
            for br, w in enumerate((woa, wob)):
                r0 = _mo(j * 48 + h * 24, 8)
                pltpu.make_async_copy(w.at[pl.ds(_mo(p * PAIR + r0, 8), 24), :],
                                      wobuf.at[slot, br, pl.ds(r0, 24), :], wosem.at[slot]).start(priority=1)

    def out_copy(b):
        r0 = _mo(b * SQ, SQ)
        return pltpu.make_async_copy(obuf.at[pl.ds(r0, SQ), :], out_hbm.at[pl.ds(r0, SQ), :], osem.at[b])

    for c in range(B * SQ // 32):
        for br, src in enumerate((xa, xb)):
            pltpu.make_async_copy(src.at[pl.ds(c * 32, 32), :], xbuf.at[0, br, pl.ds(c * 32, 32), :],
                                  xsem.at[0]).start(priority=br)
    for j in range(B):
        issue_w(0, j)
    for j in range(WLEAD):
        issue_w(1, j)
    for i in range(-6, 0):
        for t in range(NSTEP):
            issue_step(i, t)

    acc[...] = jnp.zeros(acc.shape, F32)
    otbuf[...] = jnp.zeros(otbuf.shape, F32)
    invbuf[...] = jnp.zeros(invbuf.shape, F32)

    lane = lax.broadcasted_iota(jnp.int32, (SQ, 128), 1)

    def qproj(br, n):
        r0 = _mo((n & 7) * SQ, SQ)
        q = jnp.dot(xbuf[0, br, pl.ds(r0, SQ), :], wqbuf[(n >> 3) & (NW - 1), br],
                    preferred_element_type=F32) * QSCALE
        qb = q[:, 128:256]
        qq = jnp.concatenate([q[:, 0:128], jnp.where(lane < 64, qb, 0.0),
                              jnp.where(lane >= 64, qb, 0.0), q[:, 256:384]], axis=1)
        return qq.astype(BF16)

    def oproj(br, n, ot, inv):
        r0 = _mo((n & 7) * SQ, SQ)
        o = ot.T * inv
        acc[pl.ds(r0, SQ), br * D:(br + 1) * D] += jnp.dot(
            o.astype(BF16), wobuf[(n >> 3) & (NW - 1), br], preferred_element_type=F32)

    def rows(blk, r0, nr, c0, nc):
        return jnp.concatenate([blk[:, r * SK + c0:r * SK + c0 + nc] for r in range(r0 // 8, (r0 + nr) // 8)], axis=0)

    def qk(qq, kt, hook):
        parts = []
        for h in range(2):
            for c in range(2):
                if COMPUTE:
                    parts.append(jnp.dot(qq[:, h * 256:(h + 1) * 256],
                                         rows(kt, h * 128, 256, c * 512, 512),
                                         preferred_element_type=F32))
                hook()
        if COMPUTE:
            return jnp.concatenate(parts[0:2], axis=1), jnp.concatenate(parts[2:4], axis=1)
        return None, None

    def softmax_pv(s, v):
        m = jnp.max(s, axis=-1, keepdims=True)
        p = jnp.exp2(s - m)
        l = jnp.sum(p, axis=-1, keepdims=True)
        ot = lax.dot_general(v, p.astype(BF16), NT, preferred_element_type=F32)
        return ot, jnp.broadcast_to(1.0 / l, (SQ, 128))

    def mk_inv(i1, i2):
        return jnp.concatenate([i1, jnp.where(lane < 64, i1, i2), i2], axis=1)

    wait_slot(xbuf, xsem, 0)
    wait_slot(wqbuf, wqsem, 0)
    wait_slot(wobuf, wosem, 0)
    if COMPUTE:
        qbuf[...] = qproj(0, 0)

    def body(i, carry):
        slot = i & (NBUF - 1)
        wait_slot(kvbuf, kvsem, slot)

        @pl.when(jnp.logical_and((i & 7) == 7, i < NI - 1))
        def _():
            wait_slot(wqbuf, wqsem, ((i + 1) >> 3) & (NW - 1))

        @pl.when(jnp.logical_and((i & 7) == 0, i > 0))
        def _():
            wait_slot(wobuf, wosem, (i >> 3) & (NW - 1))

        n0 = i + WLEAD
        gw = (n0 >> 3) + 1

        @pl.when(gw < NHP)
        def _():
            issue_w(gw, n0 & 7)

        step = [0]

        def hook():
            issue_step(i, step[0])
            step[0] += 1

        sa1, sa2 = qk(qbuf[...], kvbuf.at[slot, 0, 0], hook)
        if COMPUTE:
            oproj(1, jnp.maximum(i - 1, 0), otbuf[...], invbuf[...])
            ota1, ia1 = softmax_pv(sa1, rows(kvbuf.at[slot, 0, 1], 0, DH, 0, SK))
        hook()
        if COMPUTE:
            qqb = qproj(1, i)
            ota2, ia2 = softmax_pv(sa2, rows(kvbuf.at[slot, 0, 1], DH, DH, 0, SK))
        else:
            qqb = None
        hook()
        sb1, sb2 = qk(qqb, kvbuf.at[slot, 1, 0], hook)
        if COMPUTE:
            oproj(0, i, jnp.concatenate([ota1, ota2], axis=0), mk_inv(ia1, ia2))
            otb1, ib1 = softmax_pv(sb1, rows(kvbuf.at[slot, 1, 1], 0, DH, 0, SK))
        hook()
        if COMPUTE:
            qbuf[...] = qproj(0, jnp.minimum(i + 1, NI - 1))
            otb2, ib2 = softmax_pv(sb2, rows(kvbuf.at[slot, 1, 1], DH, DH, 0, SK))
        hook()
        if COMPUTE:
            otbuf[0:DH, :] = otb1
            otbuf[DH:PAIR, :] = otb2
            invbuf[...] = mk_inv(ib1, ib2)
        assert step[0] == NSTEP

        @pl.when(i > NI - B)
        def _():
            b = (i - 1) & 7
            r0 = pl.multiple_of(b * SQ, SQ)
            obuf[pl.ds(r0, SQ), :] = acc[pl.ds(r0, SQ), :].astype(BF16)

            @pl.when(i > OUT_AT)
            def _():
                out_copy(b).start()

            @pl.when(i == OUT_AT)
            def _():
                for bb in range(OUT_AT - (NI - B)):
                    out_copy(bb).start()
        return carry

    lax.fori_loop(0, NI, body, 0)

    if COMPUTE:
        oproj(1, NI - 1, otbuf[...], invbuf[...])
    obuf[(B - 1) * SQ:B * SQ, :] = acc[(B - 1) * SQ:B * SQ, :].astype(BF16)
    out_copy(B - 1).start()
    for b in range(B):
        out_copy(b).wait()


@jax.jit
def pallas_concat_heads__mha_block_cached__gqa_block_cached__near_ridge_kernel(
    A_x, A_k_cache, A_v_cache, A_wq, A_wo, B_x, B_k_cache, B_v_cache, B_wq, B_wo,
):
    def kv(a):
        a = jnp.swapaxes(a, 2, 3).reshape(B, NHP, PAIR // 8, 8, SK)
        return jnp.swapaxes(a, 2, 3).reshape(B, NHP, 8, WIDE)

    any_spec = pl.BlockSpec(memory_space=pl.ANY)
    out = pl.pallas_call(
        _kernel,
        in_specs=[any_spec] * 10,
        out_specs=any_spec,
        out_shape=jax.ShapeDtypeStruct((B * SQ, 2 * D), BF16),
        scratch_shapes=[
            pltpu.VMEM((NBUF, 2, 2, 8, WIDE), BF16),
            pltpu.VMEM((NW, 2, D, PAIR), BF16),
            pltpu.VMEM((NW, 2, PAIR, D), BF16),
            pltpu.VMEM((1, 2, B * SQ, D), BF16),
            pltpu.VMEM((B * SQ, 2 * D), F32),
            pltpu.VMEM((B * SQ, 2 * D), BF16),
            pltpu.VMEM((SQ, 512), BF16),
            pltpu.VMEM((PAIR, SQ), F32),
            pltpu.VMEM((SQ, PAIR), F32),
            pltpu.SemaphoreType.DMA((NBUF,)),
            pltpu.SemaphoreType.DMA((NW,)),
            pltpu.SemaphoreType.DMA((NW,)),
            pltpu.SemaphoreType.DMA((1,)),
            pltpu.SemaphoreType.DMA((B,)),
        ],
        compiler_params=pltpu.CompilerParams(
            vmem_limit_bytes=100 * 1024 * 1024,
        ),
    )(A_x.reshape(B * SQ, D), kv(A_k_cache), kv(A_v_cache), A_wq, A_wo,
      B_x.reshape(B * SQ, D), kv(B_k_cache), kv(B_v_cache), B_wq, B_wo)
    return out.reshape(B, SQ, 2 * D)
```

```python
import math
import jax
import jax.numpy as jnp
from jax import lax
import jax.experimental.pallas as pl
import jax.experimental.pallas.tpu as pltpu

B, SQ, D = 8, 128, 640
H, SK, DH = 32, 1024, 192
PAIR = 2 * DH
NHP = H // 2
NI = NHP * B
QSCALE = (DH ** -0.5) * math.log2(math.e)
NBUF = 8
NW = 4
NSTEP = 12
PH = 4
ROT = 6
WLEAD = 2
SH = 13
PEEL = True
I0 = 110
WAT = (0, 6)
OUT_STEP = -1
OUT_N = 5
OUTP = (1,)
F32 = jnp.float32
BF16 = jnp.bfloat16
NT = (((1,), (1,)), ((), ()))

NTILE = (PAIR // 8) * (SK // 128)
WIDE = NTILE * 128
VISITS = [[(t0, t1) for t0, t1 in ((NTILE - 16 + SH, NTILE), (0, SH)) if t1 > t0]] + [
    [(SH + 16 * k, SH + 16 * (k + 1))] for k in range(NTILE // 16 - 1)]


def _mo(x, m):
    return x if isinstance(x, int) else pl.multiple_of(x, m)


def _when(cond, fn):
    if isinstance(cond, bool):
        if cond:
            fn()
    else:
        pl.when(cond)(fn)


def _kernel(xa, ka, va, wqa, woa, xb, kb, vb, wqb, wob, out_hbm,
            kvbuf, wqbuf, wobuf, xbuf, acc, obuf, qbuf, o0buf, otbuf, invbuf,
            sems):

    class _Sem:
        def __init__(self, base):
            self.base = base

        @property
        def at(self):
            return self

        def __getitem__(self, k):
            return sems.at[self.base + k]

    kvsem, wqsem, wosem, xsem, osem = _Sem(0), _Sem(NBUF), _Sem(NBUF + NW), _Sem(NBUF + 2 * NW), _Sem(NBUF + 2 * NW + 1)

    def kv_visit(n, br, kv, k):
        slot = n & (NBUF - 1)
        src = ((ka, va), (kb, vb))[br][kv]
        return [pltpu.make_async_copy(src.at[n & 7, (n >> 3) & (NHP - 1), :, pl.ds(t0 * 128, (t1 - t0) * 128)],
                                      kvbuf.at[slot, br, kv, :, pl.ds(t0 * 128, (t1 - t0) * 128)],
                                      kvsem.at[slot]) for t0, t1 in VISITS[k]]

    def step_plan(i, t):
        vi = i + (t + PH) // NSTEP
        j = (t + PH) % NSTEP
        plan = []
        for br in range(2):
            for kv in range(2):
                for lag in (1, 0):
                    if lag == 1:
                        n = vi + 1
                        valid = (0 <= n < NI) if isinstance(n, int) else (n < NI)
                    elif isinstance(vi, int):
                        n = vi + 2 + (1 if vi < I0 else 0)
                        valid = 0 <= n < NI and vi != I0
                    else:
                        n = vi + 2 + (vi < I0).astype(jnp.int32)
                        valid = jnp.logical_and(n < NI, vi != I0)
                    plan.append((valid, n, br, kv, lag * NSTEP + (j + ROT * lag) % NSTEP, 1 - lag))
        return plan

    def issue_step(i, t):
        for valid, n, br, kv, k, prio in step_plan(i, t):
            def go(n=n, br=br, kv=kv, k=k, prio=prio):
                for c in kv_visit(n, br, kv, k):
                    c.start(priority=prio)
            _when(valid, go)

    def wait_slot(buf, sem, slot):
        pltpu.make_async_copy(buf.at[slot], buf.at[slot], sem.at[slot]).wait()

    def w_copies(g, j, h):
        p = g & (NHP - 1)
        slot = g & (NW - 1)
        qrows = pl.ds(_mo(j * 80 + h * 40, 8), 40)
        r0 = _mo(j * 48 + h * 24, 8)
        out = []
        for br in range(2):
            out.append(pltpu.make_async_copy((wqa, wqb)[br].at[qrows, pl.ds(_mo(p * PAIR, 128), PAIR)],
                                             wqbuf.at[slot, br, qrows, :], wqsem.at[slot]))
            out.append(pltpu.make_async_copy((woa, wob)[br].at[pl.ds(_mo(p * PAIR + r0, 8), 24), :],
                                             wobuf.at[slot, br, pl.ds(r0, 24), :], wosem.at[slot]))
        return out

    def issue_w(g, j, h):
        for q, c in enumerate(w_copies(g, j, h)):
            c.start(priority=q % 2)

    def out_copy(b):
        rows = pl.ds(b * SQ, SQ)
        return pltpu.make_async_copy(obuf.at[rows, :], out_hbm.at[rows, :], osem.at[b])

    def out_half(br):
        rows = pl.ds((B - 1) * SQ, SQ)
        cols = pl.ds(br * D, D)
        return pltpu.make_async_copy(obuf.at[rows, cols], out_hbm.at[rows, cols], osem.at[B - 1 + br])

    lane = lax.broadcasted_iota(jnp.int32, (SQ, 128), 1)

    def rows_of(blk, r0, nr, c0, nc):
        return jnp.concatenate(
            [blk[:, r * SK + c0:r * SK + c0 + nc] for r in range(r0 // 8, (r0 + nr) // 8)], axis=0)

    def qproj(br, n):
        x = xbuf[0, br, pl.ds(_mo((n & 7) * SQ, SQ), SQ), :]
        q = jnp.dot(x, wqbuf[(n >> 3) & (NW - 1), br], preferred_element_type=F32) * QSCALE
        qb = q[:, 128:256]
        qq = jnp.concatenate([q[:, 0:128], jnp.where(lane < 64, qb, 0.0),
                              jnp.where(lane >= 64, qb, 0.0), q[:, 256:384]], axis=1)
        return qq.astype(BF16)

    def oproj(br, n, o):
        rows = pl.ds(_mo((n & 7) * SQ, SQ), SQ)
        tot = acc[rows, br * D:(br + 1) * D] + jnp.dot(
            o, wobuf[(n >> 3) & (NW - 1), br], preferred_element_type=F32)
        acc[rows, br * D:(br + 1) * D] = tot
        obuf[rows, br * D:(br + 1) * D] = tot.astype(BF16)

    def qk(qq, kt, hook):
        parts = []
        for h in range(2):
            for c in range(2):
                parts.append(jnp.dot(qq[:, h * 256:(h + 1) * 256], rows_of(kt, h * 128, 256, c * 512, 512),
                                     preferred_element_type=F32))
                hook()
        return jnp.concatenate(parts[0:2], axis=1), jnp.concatenate(parts[2:4], axis=1)

    def softmax_pv(s, vt, h):
        m = jnp.max(s, axis=-1, keepdims=True)
        p = jnp.exp2(s - m)
        l = jnp.sum(p, axis=-1, keepdims=True)
        ot = lax.dot_general(rows_of(vt, h * DH, DH, 0, SK), p.astype(BF16), NT, preferred_element_type=F32)
        return ot, jnp.broadcast_to(1.0 / l, (SQ, 128))

    def mk_inv(i1, i2):
        return jnp.concatenate([i1, jnp.where(lane < 64, i1, i2), i2], axis=1)

    def mk_o(ot1, i1, ot2, i2):
        return (jnp.concatenate([ot1, ot2], axis=0).T * mk_inv(i1, i2)).astype(BF16)

    def carried_o():
        rest = (otbuf[...].T * invbuf[...]).astype(BF16)
        return jnp.concatenate([o0buf[...], rest], axis=1)

    xs = []
    for c in range(B * SQ // 32):
        for br, src in enumerate((xa, xb)):
            rows = pl.ds(c * 32, 32)
            xs.append([pltpu.make_async_copy(src.at[rows, :], xbuf.at[0, br, rows, :], xsem.at[0])])
    ws = [[c] for g, nj in ((0, B), (1, WLEAD)) for j in range(nj) for h in range(2) for c in w_copies(g, j, h)]
    single, paired = [], []
    for i in range(-5, 0):
        for t in range(NSTEP):
            plan = [e for e in step_plan(i, t) if e[0]]
            if len(plan) == 8:
                paired += plan
            else:
                single += [kv_visit(n, br, kv, k) for _, n, br, kv, k, _ in plan]
    merged = sorted([((q + 0.5) / len(lst), r, v) for r, lst in enumerate((xs, ws, single)) for q, v in enumerate(lst)],
                    key=lambda e: e[:2])
    for q, (_, _, v) in enumerate(merged):
        for c in v:
            c.start(priority=q % 2)
    for _, n, br, kv, k, prio in paired:
        for c in kv_visit(n, br, kv, k):
            c.start(priority=prio)

    acc[...] = jnp.zeros(acc.shape, F32)
    o0buf[...] = jnp.zeros(o0buf.shape, BF16)
    otbuf[...] = jnp.zeros(otbuf.shape, F32)
    invbuf[...] = jnp.zeros(invbuf.shape, F32)

    wait_slot(xbuf, xsem, 0)
    wait_slot(wqbuf, wqsem, 0)
    wait_slot(wobuf, wosem, 0)
    qbuf[0] = qproj(0, 0)
    qbuf[1] = qproj(1, 0)

    def body(i, carry):
        slot = i & (NBUF - 1)
        wait_slot(kvbuf, kvsem, slot)

        @pl.when(jnp.logical_and((i & 7) == 7, i < NI - 1))
        def _():
            wait_slot(wqbuf, wqsem, ((i + 1) >> 3) & (NW - 1))

        @pl.when(jnp.logical_and((i & 7) == 0, i > 0))
        def _():
            wait_slot(wobuf, wosem, (i >> 3) & (NW - 1))

        n0 = i + WLEAD
        gw = (n0 >> 3) + 1

        def w_hook(h):
            @pl.when(gw < NHP)
            def _():
                issue_w(gw, n0 & 7, h)

        step = [0]

        def hook():
            issue_step(i, step[0])
            if step[0] in WAT:
                w_hook(WAT.index(step[0]))
            if step[0] == OUT_STEP:
                @pl.when(i == NI - 2)
                def _():
                    for bb in range(OUT_N):
                        out_copy(bb).start(priority=OUTP[bb % len(OUTP)])
            step[0] += 1

        nxt = jnp.minimum(i + 1, NI - 1)
        sa1, sa2 = qk(qbuf[0], kvbuf.at[slot, 0, 0], hook)
        oproj(1, jnp.maximum(i - 1, 0), carried_o())
        ota1, ia1 = softmax_pv(sa1, kvbuf.at[slot, 0, 1], 0)
        hook()
        qbuf[0] = qproj(0, nxt)
        ota2, ia2 = softmax_pv(sa2, kvbuf.at[slot, 0, 1], 1)
        hook()
        sb1, sb2 = qk(qbuf[1], kvbuf.at[slot, 1, 0], hook)
        oproj(0, i, mk_o(ota1, ia1, ota2, ia2))
        otb1, ib1 = softmax_pv(sb1, kvbuf.at[slot, 1, 1], 0)
        hook()
        qbuf[1] = qproj(1, nxt)
        otb2, ib2 = softmax_pv(sb2, kvbuf.at[slot, 1, 1], 1)
        hook()
        o0buf[...] = (otb1[0:128, :].T * ib1).astype(BF16)
        otbuf[0:DH - 128, :] = otb1[128:DH, :]
        otbuf[DH - 128:PAIR - 128, :] = otb2
        invbuf[...] = mk_inv(ib1, ib2)[:, 128:PAIR]
        assert step[0] == NSTEP

        if not PEEL:
            @pl.when(i == NI - 2)
            def _():
                for bb in range(B - 2):
                    out_copy(bb).start()

            @pl.when(i == NI - 1)
            def _():
                out_copy(B - 2).start()
                out_half(0).start()
        return carry

    if PEEL:
        lax.fori_loop(0, NI - 1, body, 0)
        i = NI - 1
        slot = i & (NBUF - 1)
        wait_slot(kvbuf, kvsem, slot)
        for bb in range(OUT_N if OUT_STEP >= 0 else 0, B - 2):
            out_copy(bb).start(priority=OUTP[bb % len(OUTP)])
        nohook = lambda: None
        sa1, sa2 = qk(qbuf[0], kvbuf.at[slot, 0, 0], nohook)
        oproj(1, i - 1, carried_o())
        out_copy(B - 2).start(priority=OUTP[(B - 2) % len(OUTP)])
        ota1, ia1 = softmax_pv(sa1, kvbuf.at[slot, 0, 1], 0)
        sb1, sb2 = qk(qbuf[1], kvbuf.at[slot, 1, 0], nohook)
        ota2, ia2 = softmax_pv(sa2, kvbuf.at[slot, 0, 1], 1)
        otb1, ib1 = softmax_pv(sb1, kvbuf.at[slot, 1, 1], 0)
        otb2, ib2 = softmax_pv(sb2, kvbuf.at[slot, 1, 1], 1)
        oproj(0, i, mk_o(ota1, ia1, ota2, ia2))
        out_half(0).start()
        oproj(1, i, mk_o(otb1, ib1, otb2, ib2))
    else:
        lax.fori_loop(0, NI, body, 0)
        oproj(1, NI - 1, carried_o())
    out_half(1).start()
    for b in range(B - 1):
        out_copy(b).wait()
    out_half(0).wait()
    out_half(1).wait()


@jax.jit
def pallas_concat_heads__mha_block_cached__gqa_block_cached__near_ridge_kernel(
    A_x, A_k_cache, A_v_cache, A_wq, A_wo, B_x, B_k_cache, B_v_cache, B_wq, B_wo,
):
    def kv(a):
        a = jnp.swapaxes(a, 2, 3).reshape(B, NHP, PAIR // 8, 8, SK)
        return jnp.swapaxes(a, 2, 3).reshape(B, NHP, 8, WIDE)

    any_spec = pl.BlockSpec(memory_space=pl.ANY)
    out = pl.pallas_call(
        _kernel,
        in_specs=[any_spec] * 10,
        out_specs=any_spec,
        out_shape=jax.ShapeDtypeStruct((B * SQ, 2 * D), BF16),
        scratch_shapes=[
            pltpu.VMEM((NBUF, 2, 2, 8, WIDE), BF16),
            pltpu.VMEM((NW, 2, D, PAIR), BF16),
            pltpu.VMEM((NW, 2, PAIR, D), BF16),
            pltpu.VMEM((1, 2, B * SQ, D), BF16),
            pltpu.VMEM((B * SQ, 2 * D), F32),
            pltpu.VMEM((B * SQ, 2 * D), BF16),
            pltpu.VMEM((2, SQ, 512), BF16),
            pltpu.VMEM((SQ, 128), BF16),
            pltpu.VMEM((PAIR - 128, SQ), F32),
            pltpu.VMEM((SQ, PAIR - 128), F32),
            pltpu.SemaphoreType.DMA((NBUF + 2 * NW + 1 + B + 1,)),
        ],
        compiler_params=pltpu.CompilerParams(
            vmem_limit_bytes=100 * 1024 * 1024,
            disable_semaphore_checks=True,
        ),
    )(A_x.reshape(B * SQ, D), kv(A_k_cache), kv(A_v_cache), A_wq, A_wo,
      B_x.reshape(B * SQ, D), kv(B_k_cache), kv(B_v_cache), B_wq, B_wo)
    return out.reshape(B, SQ, 2 * D)
```

```python
import math
import jax
import jax.numpy as jnp
from jax import lax
import jax.experimental.pallas as pl
import jax.experimental.pallas.tpu as pltpu

B, SQ, D = 8, 128, 640
H, SK, DH = 32, 1024, 192
PAIR = 2 * DH
NHP = H // 2
NI = NHP * B
QSCALE = (DH ** -0.5) * math.log2(math.e)
NBUF = 8
NW = 4
NSTEP = 12
PH = 4
I0 = 110
ROT = 6
WAT = (0, 6)
WLEAD = 2
WQ0 = 8
SH = 13
F32 = jnp.float32
BF16 = jnp.bfloat16
NT = (((1,), (1,)), ((), ()))

QRT = D // 8
NTILE = (PAIR // 8) * (SK // 128)
WIDE = NTILE * 128
_CUTS = [0] + [SH + 16 * k for k in range(NTILE // 16 - 1)] + [NTILE]
VISITS = list(zip(_CUTS[:-1], _CUTS[1:]))
KVSEM, WOSEM, WQSEM, XSEM, OSEM = 0, NBUF, NBUF + NW, NBUF + NW + 4, NBUF + NW + 5
NSEM = OSEM + B + 1


def _mo(x, m):
    return x if isinstance(x, int) else pl.multiple_of(x, m)


def _pair_of(g):
    return (g + (NHP - 1)) & (NHP - 1)


def _kernel(xa, ka, va, wqa, woa, xb, kb, vb, wqb, wob, out_hbm,
            kvbuf, wqbuf, wobuf, xbuf, acc, obuf, qbuf, o0buf, otbuf, invbuf, sems):

    def wait_all(ref, sem):
        pltpu.make_async_copy(ref, ref, sems.at[sem]).wait()

    def kv_copy(n, br, kv, k):
        t0, t1 = VISITS[k]
        cols = pl.ds(t0 * 128, (t1 - t0) * 128)
        slot = n & (NBUF - 1)
        src = ((ka, va), (kb, vb))[br][kv]
        return pltpu.make_async_copy(src.at[n & 7, _pair_of(n >> 3), :, cols],
                                     kvbuf.at[slot, br, kv, :, cols], sems.at[KVSEM + slot])

    def step_plan(i, t):
        vi = i + (t + PH) // NSTEP
        j = (t + PH) % NSTEP
        n1 = vi + 1
        if isinstance(vi, int):
            n0 = vi + 2 + (1 if vi < I0 else 0)
            ok1, ok0 = 0 <= n1 < NI, 0 <= n0 < NI and vi != I0
        else:
            n0 = vi + 2 + (vi < I0).astype(jnp.int32)
            ok1, ok0 = n1 < NI, jnp.logical_and(n0 < NI, vi != I0)
        plan = []
        for br in range(2):
            for kv in range(2):
                plan.append((ok1, (n1, br, kv, NSTEP + (j + ROT) % NSTEP), 0))
                plan.append((ok0, (n0, br, kv, j), 1))
        return plan

    def wo_copies(g, j, h):
        slot = g & (NW - 1)
        r0 = _mo(j * 48 + h * 24, 8)
        return [pltpu.make_async_copy(w.at[pl.ds(_mo(_pair_of(g) * PAIR + r0, 8), 24), :],
                                      wobuf.at[slot, br, pl.ds(r0, 24), :], sems.at[WOSEM + slot])
                for br, w in enumerate((woa, wob))]

    def wq_cols(g):
        return pl.ds(_mo((SH + 16 * g) * 128, 128), 2048)

    def wq_copies(w):
        if isinstance(w, int):
            g, r = divmod(w, QRT)
        else:
            g = (w >= QRT).astype(jnp.int32)
            r = jnp.minimum(w - g * QRT, QRT - 1)
        rows = pl.ds(_mo(r * 8, 8), 8)
        return [pltpu.make_async_copy(w_.at[rows, wq_cols(g)], wqbuf.at[br, rows, wq_cols(g)],
                                      sems.at[WQSEM + 2 + g]) for br, w_ in enumerate((wqa, wqb))]

    wq_lo = pl.ds(0, SH * 128)
    wq_hi = pl.ds((32 + SH) * 128, (16 - SH) * 128)

    def wq0_copies(br, r):
        out = []
        for rr, cols, sm in ((r - 1, wq_hi, 1), (r, wq_lo, 0)):
            if 0 <= rr < QRT:
                rows = pl.ds(rr * 8, 8)
                out.append(pltpu.make_async_copy((wqa, wqb)[br].at[rows, cols], wqbuf.at[br, rows, cols],
                                                 sems.at[WQSEM + sm]))
        return out

    def out_copy(b):
        rows = pl.ds(b * SQ, SQ)
        return pltpu.make_async_copy(obuf.at[rows, :], out_hbm.at[rows, :], sems.at[OSEM + b])

    def out_half(br):
        rows = pl.ds((B - 1) * SQ, SQ)
        cols = pl.ds(br * D, D)
        return pltpu.make_async_copy(obuf.at[rows, cols], out_hbm.at[rows, cols], sems.at[OSEM + B - 1 + br])

    lane = lax.broadcasted_iota(jnp.int32, (SQ, 128), 1)

    def rows_of(blk, r0, nr, c0, nc):
        return jnp.concatenate(
            [blk[:, r * SK + c0:r * SK + c0 + nc] for r in range(r0 // 8, (r0 + nr) // 8)], axis=0)

    def qproj(br, n):
        x = xbuf[br, pl.ds(_mo((n & 7) * SQ, SQ), SQ), :]
        wq = wqbuf[br, :, pl.ds(_mo(_pair_of(n >> 3) * PAIR, 128), PAIR)]
        q = jnp.dot(x, wq, preferred_element_type=F32) * QSCALE
        qb = q[:, 128:256]
        qq = jnp.concatenate([q[:, 0:128], jnp.where(lane < 64, qb, 0.0),
                              jnp.where(lane >= 64, qb, 0.0), q[:, 256:384]], axis=1)
        qbuf[br] = qq.astype(BF16)

    def oproj(br, n, o):
        rows = pl.ds(_mo((n & 7) * SQ, SQ), SQ)
        tot = acc[rows, br * D:(br + 1) * D] + jnp.dot(
            o, wobuf[(n >> 3) & (NW - 1), br], preferred_element_type=F32)
        acc[rows, br * D:(br + 1) * D] = tot
        obuf[rows, br * D:(br + 1) * D] = tot.astype(BF16)

    def qk(br, slot, hook):
        qq = qbuf[br]
        kt = kvbuf.at[slot, br, 0]
        parts = []
        for h in range(2):
            for c in range(2):
                parts.append(jnp.dot(qq[:, h * 256:(h + 1) * 256], rows_of(kt, h * 128, 256, c * 512, 512),
                                     preferred_element_type=F32))
                hook()
        return jnp.concatenate(parts[0:2], axis=1), jnp.concatenate(parts[2:4], axis=1)

    def softmax_pv(s, br, slot, h):
        m = jnp.max(s, axis=-1, keepdims=True)
        p = jnp.exp2(s - m)
        l = jnp.sum(p, axis=-1, keepdims=True)
        vt = rows_of(kvbuf.at[slot, br, 1], h * DH, DH, 0, SK)
        ot = lax.dot_general(vt, p.astype(BF16), NT, preferred_element_type=F32)
        return ot, jnp.broadcast_to(1.0 / l, (SQ, 128))

    def mk_inv(i1, i2):
        return jnp.concatenate([i1, jnp.where(lane < 64, i1, i2), i2], axis=1)

    def mk_o(ot1, i1, ot2, i2):
        return (jnp.concatenate([ot1, ot2], axis=0).T * mk_inv(i1, i2)).astype(BF16)

    def carried_o():
        rest = (otbuf[...].T * invbuf[...]).astype(BF16)
        return jnp.concatenate([o0buf[...], rest], axis=1)

    xs = [[pltpu.make_async_copy(src.at[pl.ds(c * 32, 32), :], xbuf.at[br, pl.ds(c * 32, 32), :], sems.at[XSEM])]
          for c in range(B * SQ // 32) for br, src in enumerate((xa, xb))]
    wos = [[c] for g, nj in ((0, B), (1, WLEAD)) for j in range(nj) for h in range(2) for c in wo_copies(g, j, h)]
    wqs = [wq0_copies(br, r) for r in range(QRT + 1) for br in range(2)]
    wqs += [[c] for w in range(WQ0) for c in wq_copies(w)]
    single, paired = [], []
    for i in range(-5, 0):
        for t in range(NSTEP):
            plan = [e for e in step_plan(i, t) if e[0]]
            if len(plan) == 8:
                paired += plan
            else:
                single += [[kv_copy(*args)] for _, args, _ in plan]
    merged = sorted([((q + 0.5) / len(lst), r, q) for r, lst in enumerate((xs, wos, wqs, single))
                     for q in range(len(lst))])
    for pos, (_, r, q) in enumerate(merged):
        for c in (xs, wos, wqs, single)[r][q]:
            c.start(priority=pos % 2)
    for _, args, prio in paired:
        kv_copy(*args).start(priority=prio)

    acc[...] = jnp.zeros(acc.shape, F32)
    o0buf[...] = jnp.zeros(o0buf.shape, BF16)
    otbuf[...] = jnp.zeros(otbuf.shape, F32)
    invbuf[...] = jnp.zeros(invbuf.shape, F32)

    wait_all(xbuf, XSEM)
    wait_all(wqbuf.at[:, :, wq_lo], WQSEM)
    wait_all(wqbuf.at[:, :, wq_hi], WQSEM + 1)
    wait_all(wobuf.at[0], WOSEM)
    qproj(0, 0)
    qproj(1, 0)

    def body(i, carry):
        slot = i & (NBUF - 1)
        wait_all(kvbuf.at[slot], KVSEM + slot)

        for g in range(2):
            @pl.when(i == ((SH + 16 * g) // 3 + 1) * B - 1)
            def _(g=g):
                wait_all(wqbuf.at[:, :, wq_cols(g)], WQSEM + 2 + g)

        @pl.when(jnp.logical_and((i & 7) == 0, i > 0))
        def _():
            ws = (i >> 3) & (NW - 1)
            wait_all(wobuf.at[ws], WOSEM + ws)

        step = [0]

        def hook():
            t = step[0]
            step[0] += 1
            for ok, args, prio in step_plan(i, t):
                @pl.when(ok)
                def _(args=args, prio=prio):
                    kv_copy(*args).start(priority=prio)
            if t in WAT:
                h = WAT.index(t)
                gw = ((i + WLEAD) >> 3) + 1
                w = WQ0 + 2 * i + h

                @pl.when(gw < NHP)
                def _():
                    for q, c in enumerate(wo_copies(gw, (i + WLEAD) & 7, h)):
                        c.start(priority=q)

                @pl.when(w < 2 * QRT)
                def _():
                    for q, c in enumerate(wq_copies(w)):
                        c.start(priority=q)

        sa1, sa2 = qk(0, slot, hook)
        oproj(1, jnp.maximum(i - 1, 0), carried_o())
        ota1, ia1 = softmax_pv(sa1, 0, slot, 0)
        hook()
        qproj(0, i + 1)
        ota2, ia2 = softmax_pv(sa2, 0, slot, 1)
        hook()
        sb1, sb2 = qk(1, slot, hook)
        oproj(0, i, mk_o(ota1, ia1, ota2, ia2))
        otb1, ib1 = softmax_pv(sb1, 1, slot, 0)
        hook()
        qproj(1, i + 1)
        otb2, ib2 = softmax_pv(sb2, 1, slot, 1)
        hook()
        o0buf[...] = (otb1[0:128, :].T * ib1).astype(BF16)
        otbuf[0:DH - 128, :] = otb1[128:DH, :]
        otbuf[DH - 128:PAIR - 128, :] = otb2
        invbuf[...] = mk_inv(ib1, ib2)[:, 128:PAIR]
        assert step[0] == NSTEP
        return carry

    lax.fori_loop(0, NI - 1, body, 0)

    i = NI - 1
    slot = i & (NBUF - 1)
    wait_all(kvbuf.at[slot], KVSEM + slot)
    for b in range(B - 2):
        out_copy(b).start(priority=1)

    def nohook():
        pass

    sa1, sa2 = qk(0, slot, nohook)
    oproj(1, i - 1, carried_o())
    out_copy(B - 2).start(priority=1)
    ota1, ia1 = softmax_pv(sa1, 0, slot, 0)
    sb1, sb2 = qk(1, slot, nohook)
    ota2, ia2 = softmax_pv(sa2, 0, slot, 1)
    otb1, ib1 = softmax_pv(sb1, 1, slot, 0)
    otb2, ib2 = softmax_pv(sb2, 1, slot, 1)
    oproj(0, i, mk_o(ota1, ia1, ota2, ia2))
    out_half(0).start()
    oproj(1, i, mk_o(otb1, ib1, otb2, ib2))
    out_half(1).start()
    for b in range(B - 1):
        out_copy(b).wait()
    out_half(0).wait()
    out_half(1).wait()


@jax.jit
def pallas_concat_heads__mha_block_cached__gqa_block_cached__near_ridge_kernel(
    A_x, A_k_cache, A_v_cache, A_wq, A_wo, B_x, B_k_cache, B_v_cache, B_wq, B_wo,
):
    def kv(a):
        a = jnp.swapaxes(a, 2, 3).reshape(B, NHP, PAIR // 8, 8, SK)
        return jnp.swapaxes(a, 2, 3).reshape(B, NHP, 8, WIDE)

    any_spec = pl.BlockSpec(memory_space=pl.ANY)
    out = pl.pallas_call(
        _kernel,
        in_specs=[any_spec] * 10,
        out_specs=any_spec,
        out_shape=jax.ShapeDtypeStruct((B * SQ, 2 * D), BF16),
        scratch_shapes=[
            pltpu.VMEM((NBUF, 2, 2, 8, WIDE), BF16),
            pltpu.VMEM((2, D, H * DH), BF16),
            pltpu.VMEM((NW, 2, PAIR, D), BF16),
            pltpu.VMEM((2, B * SQ, D), BF16),
            pltpu.VMEM((B * SQ, 2 * D), F32),
            pltpu.VMEM((B * SQ, 2 * D), BF16),
            pltpu.VMEM((2, SQ, 512), BF16),
            pltpu.VMEM((SQ, 128), BF16),
            pltpu.VMEM((PAIR - 128, SQ), F32),
            pltpu.VMEM((SQ, PAIR - 128), F32),
            pltpu.SemaphoreType.DMA((NSEM,)),
        ],
        compiler_params=pltpu.CompilerParams(
            vmem_limit_bytes=100 * 1024 * 1024,
            disable_semaphore_checks=True,
        ),
    )(A_x.reshape(B * SQ, D), kv(A_k_cache), kv(A_v_cache), A_wq, A_wo,
      B_x.reshape(B * SQ, D), kv(B_k_cache), kv(B_v_cache), B_wq, B_wo)
    return out.reshape(B, SQ, 2 * D)
```

```python
import math
import jax
import jax.numpy as jnp
from jax import lax
import jax.experimental.pallas as pl
import jax.experimental.pallas.tpu as pltpu

B, SQ, D = 8, 128, 640
H, SK, DH = 32, 1024, 192
PAIR = 2 * DH
NHP = H // 2
NI = NHP * B
QSCALE = (DH ** -0.5) * math.log2(math.e)
NBUF = 8
NW = 4
NSTEP = 12
PH = 5
I0 = 105
ROT = 3
WAT = (0, 6)
QAT = (1, 3, 5, 7, 9)
WLEAD = 2
OCH = 16
SH = 13
F32 = jnp.float32
BF16 = jnp.bfloat16
NT = (((1,), (1,)), ((), ()))

assert 12 <= SH <= 13
QRT = D // 8
NTILE = (PAIR // 8) * (SK // 128)
WIDE = NTILE * 128
_CUTS = [0] + [SH + 16 * k for k in range(NTILE // 16 - 1)] + [NTILE]
VISITS = list(zip(_CUTS[:-1], _CUTS[1:]))
KVSEM, WOSEM, WQSEM, XSEM, OSEM = 0, NBUF, NBUF + NW, NBUF + NW + 4, NBUF + NW + 5
NSEM = OSEM + B + 1


def _mo(x, m):
    return x if isinstance(x, int) else pl.multiple_of(x, m)


def _pair_of(g):
    return (g + (NHP - 1)) & (NHP - 1)


def _kernel(xa, ka, va, wqa, woa, xb, kb, vb, wqb, wob, out_hbm,
            kvbuf, wqbuf, wobuf, xbuf, acc, obuf, qbuf, o0buf, otbuf, invbuf, sems):

    def wait_all(ref, sem):
        pltpu.make_async_copy(ref, ref, sems.at[sem]).wait()

    def kv_copy(n, br, kv, k):
        t0, t1 = VISITS[k]
        cols = pl.ds(t0 * 128, (t1 - t0) * 128)
        slot = n & (NBUF - 1)
        src = ((ka, va), (kb, vb))[br][kv]
        return pltpu.make_async_copy(src.at[n & 7, _pair_of(n >> 3), :, cols],
                                     kvbuf.at[slot, br, kv, :, cols], sems.at[KVSEM + slot])

    def step_plan(i, t):
        vi = i + (t + PH) // NSTEP
        m, br = divmod((t + PH) % NSTEP, 2)
        n1 = vi + 1
        if isinstance(vi, int):
            n0 = vi + 2 + (1 if vi < I0 else 0)
            ok1, ok0 = 0 <= n1 < NI, 0 <= n0 < NI and vi != I0
        else:
            n0 = vi + 2 + (vi < I0).astype(jnp.int32)
            ok1, ok0 = n1 < NI, jnp.logical_and(n0 < NI, vi != I0)
        late = [(n1, br, kv, 11 + 2 * ((m + ROT) % 6) + h) for kv in range(2) for h in range(2)]
        if m == 0:
            early = [(n0, b2, kv, (0, 23)[br]) for b2 in range(2) for kv in range(2)]
        else:
            early = [(n0, br, kv, 2 * m - 1 + h) for kv in range(2) for h in range(2)]
        plan = []
        for a1, a0 in zip(late, early):
            plan.append((ok1, a1, 0))
            plan.append((ok0, a0, 1))
        return plan

    def wo_copies(g, j, h):
        slot = g & (NW - 1)
        r0 = _mo(j * 48 + h * 24, 8)
        return [pltpu.make_async_copy(w.at[pl.ds(_mo(_pair_of(g) * PAIR + r0, 8), 24), :],
                                      wobuf.at[slot, br, pl.ds(r0, 24), :], sems.at[WOSEM + slot])
                for br, w in enumerate((woa, wob))]

    def wq_cols(g):
        return pl.ds(_mo((SH + 16 * g) * 128, 128), 2048)

    def wq_copies(i, k):
        g = (i >> 5) & 1
        rows = pl.ds(pl.multiple_of((((i >> 1) & 15) * 5 + k) * 8, 8), 8)
        return [pltpu.make_async_copy(w.at[rows, wq_cols(g)], wqbuf.at[br, rows, wq_cols(g)],
                                      sems.at[WQSEM + 2 + g]) for br, w in enumerate((wqa, wqb))]

    wq_lo = pl.ds(0, SH * 128)
    wq_hi = pl.ds((32 + SH) * 128, (16 - SH) * 128)

    def wq0_copies(br, r):
        out = []
        for rr, cols, sm in ((r - 1, wq_hi, 1), (r, wq_lo, 0)):
            if 0 <= rr < QRT:
                rows = pl.ds(rr * 8, 8)
                out.append(pltpu.make_async_copy((wqa, wqb)[br].at[rows, cols], wqbuf.at[br, rows, cols],
                                                 sems.at[WQSEM + sm]))
        return out

    def out_copy(r0, nr, c0, nc, sem):
        rows, cols = pl.ds(r0, nr), pl.ds(c0, nc)
        return pltpu.make_async_copy(obuf.at[rows, cols], out_hbm.at[rows, cols], sems.at[OSEM + sem])

    lane = lax.broadcasted_iota(jnp.int32, (SQ, 128), 1)

    def rows_of(blk, r0, nr, c0, nc):
        return jnp.concatenate(
            [blk[:, r * SK + c0:r * SK + c0 + nc] for r in range(r0 // 8, (r0 + nr) // 8)], axis=0)

    def qproj(br, n):
        x = xbuf[br, pl.ds(_mo((n & 7) * SQ, SQ), SQ), :]
        wq = wqbuf[br, :, pl.ds(_mo(_pair_of(n >> 3) * PAIR, 128), PAIR)]
        q = jnp.dot(x, wq, preferred_element_type=F32) * QSCALE
        qb = q[:, 128:256]
        qq = jnp.concatenate([q[:, 0:128], jnp.where(lane < 64, qb, 0.0),
                              jnp.where(lane >= 64, qb, 0.0), q[:, 256:384]], axis=1)
        qbuf[n & 1, br] = qq.astype(BF16)

    def oproj(br, n, o):
        rows = pl.ds(_mo((n & 7) * SQ, SQ), SQ)
        tot = acc[rows, br * D:(br + 1) * D] + jnp.dot(
            o, wobuf[(n >> 3) & (NW - 1), br], preferred_element_type=F32)
        acc[rows, br * D:(br + 1) * D] = tot
        obuf[rows, br * D:(br + 1) * D] = tot.astype(BF16)

    def qk(br, n, hook):
        qq = qbuf[n & 1, br]
        kt = kvbuf.at[n & (NBUF - 1), br, 0]
        parts = []
        for h in range(2):
            for c in range(2):
                parts.append(jnp.dot(qq[:, h * 256:(h + 1) * 256], rows_of(kt, h * 128, 256, c * 512, 512),
                                     preferred_element_type=F32))
                hook()
        return jnp.concatenate(parts[0:2], axis=1), jnp.concatenate(parts[2:4], axis=1)

    def softmax_pv(s, br, n, h):
        m = jnp.max(s, axis=-1, keepdims=True)
        p = jnp.exp2(s - m)
        l = jnp.sum(p, axis=-1, keepdims=True)
        vt = rows_of(kvbuf.at[n & (NBUF - 1), br, 1], h * DH, DH, 0, SK)
        ot = lax.dot_general(vt, p.astype(BF16), NT, preferred_element_type=F32)
        return ot, jnp.broadcast_to(1.0 / l, (SQ, 128))

    def mk_inv(i1, i2):
        return jnp.concatenate([i1, jnp.where(lane < 64, i1, i2), i2], axis=1)

    def mk_o(ot1, i1, ot2, i2):
        return (jnp.concatenate([ot1, ot2], axis=0).T * mk_inv(i1, i2)).astype(BF16)

    def carried_o():
        rest = (otbuf[...].T * invbuf[...]).astype(BF16)
        return jnp.concatenate([o0buf[...], rest], axis=1)

    xs = [[pltpu.make_async_copy(src.at[pl.ds(c * 32, 32), :], xbuf.at[br, pl.ds(c * 32, 32), :], sems.at[XSEM])]
          for c in range(B * SQ // 32) for br, src in enumerate((xa, xb))]
    wos = [[c] for g, nj in ((0, B), (1, WLEAD)) for j in range(nj) for h in range(2) for c in wo_copies(g, j, h)]
    wqs = [wq0_copies(br, r) for r in range(QRT + 1) for br in range(2)]
    single, paired = [], []
    for i in range(-5, 0):
        for t in range(NSTEP):
            plan = [e for e in step_plan(i, t) if e[0]]
            if len(plan) == 8:
                paired += plan
            else:
                single += [[kv_copy(*args)] for _, args, _ in plan]
    merged = sorted([((q + 0.5) / len(lst), r, q) for r, lst in enumerate((xs, wos, wqs, single))
                     for q in range(len(lst))])
    for pos, (_, r, q) in enumerate(merged):
        for c in (xs, wos, wqs, single)[r][q]:
            c.start(priority=pos % 2)
    for _, args, prio in paired:
        kv_copy(*args).start(priority=prio)

    acc[...] = jnp.zeros(acc.shape, F32)
    o0buf[...] = jnp.zeros(o0buf.shape, BF16)
    otbuf[...] = jnp.zeros(otbuf.shape, F32)
    invbuf[...] = jnp.zeros(invbuf.shape, F32)

    wait_all(xbuf, XSEM)
    wait_all(wqbuf.at[:, :, wq_lo], WQSEM)
    wait_all(wqbuf.at[:, :, wq_hi], WQSEM + 1)
    wait_all(wobuf.at[0], WOSEM)
    for n in range(2):
        qproj(0, n)
        qproj(1, n)

    def body(i, carry):
        slot = i & (NBUF - 1)
        wait_all(kvbuf.at[slot], KVSEM + slot)

        for g in range(2):
            @pl.when(i == ((SH + 16 * g) // 3 + 1) * B - 2)
            def _(g=g):
                wait_all(wqbuf.at[:, :, wq_cols(g)], WQSEM + 2 + g)

        @pl.when(jnp.logical_and((i & 7) == 0, i > 0))
        def _():
            ws = (i >> 3) & (NW - 1)
            wait_all(wobuf.at[ws], WOSEM + ws)

        step = [0]

        def hook():
            t = step[0]
            step[0] += 1
            for ok, args, prio in step_plan(i, t):
                @pl.when(ok)
                def _(args=args, prio=prio):
                    kv_copy(*args).start(priority=prio)
            if t in WAT:
                gw = ((i + WLEAD) >> 3) + 1

                @pl.when(gw < NHP)
                def _():
                    for q, c in enumerate(wo_copies(gw, (i + WLEAD) & 7, WAT.index(t))):
                        c.start(priority=q)
            if t in QAT:
                @pl.when(jnp.logical_and(i < 64, (i & 1) == 0))
                def _():
                    for q, c in enumerate(wq_copies(i, QAT.index(t))):
                        c.start(priority=q)

        sa1, sa2 = qk(0, i, hook)
        oproj(1, jnp.maximum(i - 1, 0), carried_o())
        ota1, ia1 = softmax_pv(sa1, 0, i, 0)
        hook()
        qproj(0, i + 2)
        ota2, ia2 = softmax_pv(sa2, 0, i, 1)
        hook()
        sb1, sb2 = qk(1, i, hook)
        oproj(0, i, mk_o(ota1, ia1, ota2, ia2))
        otb1, ib1 = softmax_pv(sb1, 1, i, 0)
        hook()
        qproj(1, i + 2)
        otb2, ib2 = softmax_pv(sb2, 1, i, 1)
        hook()
        o0buf[...] = (otb1[0:128, :].T * ib1).astype(BF16)
        otbuf[0:DH - 128, :] = otb1[128:DH, :]
        otbuf[DH - 128:PAIR - 128, :] = otb2
        invbuf[...] = mk_inv(ib1, ib2)[:, 128:PAIR]
        assert step[0] == NSTEP
        return carry

    lax.fori_loop(0, NI - 2, body, 0)

    for i in (NI - 2, NI - 1):
        wait_all(kvbuf.at[i & (NBUF - 1)], KVSEM + (i & (NBUF - 1)))
        if i == NI - 1:
            for c in range(SQ // OCH):
                for b in range(B - 1):
                    out_copy(b * SQ + c * OCH, OCH, 0, 2 * D, b).start(priority=(c + b) % 2)
        tail_step = [0]

        def tail_hook():
            for ok, args, prio in step_plan(i, tail_step[0]):
                if ok:
                    kv_copy(*args).start(priority=prio)
            tail_step[0] += 1

        sa1, sa2 = qk(0, i, tail_hook)
        if i == NI - 2:
            oproj(1, i - 1, carried_o())
            ota1, ia1 = softmax_pv(sa1, 0, i, 0)
            tail_hook()
            sb1, sb2 = qk(1, i, tail_hook)
        else:
            sb1, sb2 = qk(1, i, tail_hook)
            ota1, ia1 = softmax_pv(sa1, 0, i, 0)
            tail_hook()
        ota2, ia2 = softmax_pv(sa2, 0, i, 1)
        tail_hook()
        otb1, ib1 = softmax_pv(sb1, 1, i, 0)
        tail_hook()
        otb2, ib2 = softmax_pv(sb2, 1, i, 1)
        tail_hook()
        assert tail_step[0] == NSTEP
        oproj(0, i, mk_o(ota1, ia1, ota2, ia2))
        if i == NI - 1:
            out_copy((B - 1) * SQ, SQ, 0, D, B - 1).start()
        oproj(1, i, mk_o(otb1, ib1, otb2, ib2))
    out_copy((B - 1) * SQ, SQ, D, D, B).start()
    for b in range(B - 1):
        out_copy(b * SQ, SQ, 0, 2 * D, b).wait()
    out_copy((B - 1) * SQ, SQ, 0, D, B - 1).wait()
    out_copy((B - 1) * SQ, SQ, D, D, B).wait()


@jax.jit
def pallas_concat_heads__mha_block_cached__gqa_block_cached__near_ridge_kernel(
    A_x, A_k_cache, A_v_cache, A_wq, A_wo, B_x, B_k_cache, B_v_cache, B_wq, B_wo,
):
    def kv(a):
        a = jnp.swapaxes(a, 2, 3).reshape(B, NHP, PAIR // 8, 8, SK)
        return jnp.swapaxes(a, 2, 3).reshape(B, NHP, 8, WIDE)

    any_spec = pl.BlockSpec(memory_space=pl.ANY)
    out = pl.pallas_call(
        _kernel,
        in_specs=[any_spec] * 10,
        out_specs=any_spec,
        out_shape=jax.ShapeDtypeStruct((B * SQ, 2 * D), BF16),
        scratch_shapes=[
            pltpu.VMEM((NBUF, 2, 2, 8, WIDE), BF16),
            pltpu.VMEM((2, D, H * DH), BF16),
            pltpu.VMEM((NW, 2, PAIR, D), BF16),
            pltpu.VMEM((2, B * SQ, D), BF16),
            pltpu.VMEM((B * SQ, 2 * D), F32),
            pltpu.VMEM((B * SQ, 2 * D), BF16),
            pltpu.VMEM((2, 2, SQ, 512), BF16),
            pltpu.VMEM((SQ, 128), BF16),
            pltpu.VMEM((PAIR - 128, SQ), F32),
            pltpu.VMEM((SQ, PAIR - 128), F32),
            pltpu.SemaphoreType.DMA((NSEM,)),
        ],
        compiler_params=pltpu.CompilerParams(
            vmem_limit_bytes=100 * 1024 * 1024,
            disable_semaphore_checks=True,
        ),
    )(A_x.reshape(B * SQ, D), kv(A_k_cache), kv(A_v_cache), A_wq, A_wo,
      B_x.reshape(B * SQ, D), kv(B_k_cache), kv(B_v_cache), B_wq, B_wo)
    return out.reshape(B, SQ, 2 * D)
```

```python
import math
import jax
import jax.numpy as jnp
from jax import lax
import jax.experimental.pallas as pl
import jax.experimental.pallas.tpu as pltpu

B, SQ, D = 8, 128, 640
H, SK, DH = 32, 1024, 192
PAIR = 2 * DH
NHP = H // 2
NI = NHP * B
QSCALE = (DH ** -0.5) * math.log2(math.e)
NBUF = 8
NW = 4
NSTEP = 12
PH = 5
I0 = 105
ROT = 3
WAT = (0, 6)
QAT = (1, 3, 5, 7, 9)
WLEAD = 2
OCH = 16
SH = 13
F32 = jnp.float32
BF16 = jnp.bfloat16
NT = (((1,), (1,)), ((), ()))

assert 12 <= SH <= 13
QRT = D // 8
NTILE = (PAIR // 8) * (SK // 128)
WIDE = NTILE * 128
_CUTS = [0] + [SH + 16 * k for k in range(NTILE // 16 - 1)] + [NTILE]
VISITS = list(zip(_CUTS[:-1], _CUTS[1:]))
KVSEM, WOSEM, WQSEM, XSEM, OSEM = 0, NBUF, NBUF + NW, NBUF + NW + 4, NBUF + NW + 5
NSEM = OSEM + 1


def _mo(x, m):
    return x if isinstance(x, int) else pl.multiple_of(x, m)


def _pair_of(g):
    return (g + (NHP - 1)) & (NHP - 1)


def _kernel(xa, ka, va, wqa, woa, xb, kb, vb, wqb, wob, out_hbm,
            kvbuf, wqbuf, wobuf, xbuf, acc, obuf, qbuf, o0buf, otbuf, invbuf, sems):

    def wait_all(ref, sem):
        pltpu.make_async_copy(ref, ref, sems.at[sem]).wait()

    def kv_copy(n, br, kv, k):
        t0, t1 = VISITS[k]
        cols = pl.ds(t0 * 128, (t1 - t0) * 128)
        slot = n & (NBUF - 1)
        src = ((ka, va), (kb, vb))[br][kv]
        return pltpu.make_async_copy(src.at[n & 7, _pair_of(n >> 3), :, cols],
                                     kvbuf.at[slot, br, kv, :, cols], sems.at[KVSEM + slot])

    def step_plan(i, t):
        vi = i + (t + PH) // NSTEP
        m, br = divmod((t + PH) % NSTEP, 2)
        n1 = vi + 1
        if isinstance(vi, int):
            n0 = vi + 2 + (1 if vi < I0 else 0)
            ok1, ok0 = 0 <= n1 < NI, 0 <= n0 < NI and vi != I0
        else:
            n0 = vi + 2 + (vi < I0).astype(jnp.int32)
            ok1, ok0 = n1 < NI, jnp.logical_and(n0 < NI, vi != I0)
        late = [(n1, br, kv, 11 + 2 * ((m + ROT) % 6) + h) for kv in range(2) for h in range(2)]
        if m == 0:
            early = [(n0, b2, kv, (0, 23)[br]) for b2 in range(2) for kv in range(2)]
        else:
            early = [(n0, br, kv, 2 * m - 1 + h) for kv in range(2) for h in range(2)]
        plan = []
        for a1, a0 in zip(late, early):
            plan.append((ok1, a1, 0))
            plan.append((ok0, a0, 1))
        return plan

    def wo_copies(g, j, h):
        slot = g & (NW - 1)
        r0 = _mo(j * 48 + h * 24, 8)
        return [pltpu.make_async_copy(w.at[pl.ds(_mo(_pair_of(g) * PAIR + r0, 8), 24), :],
                                      wobuf.at[slot, br, pl.ds(r0, 24), :], sems.at[WOSEM + slot])
                for br, w in enumerate((woa, wob))]

    def wq_cols(g):
        return pl.ds(_mo((SH + 16 * g) * 128, 128), 2048)

    def wq_copies(i, k):
        g = (i >> 5) & 1
        rows = pl.ds(pl.multiple_of((((i >> 1) & 15) * 5 + k) * 8, 8), 8)
        return [pltpu.make_async_copy(w.at[rows, wq_cols(g)], wqbuf.at[br, rows, wq_cols(g)],
                                      sems.at[WQSEM + 2 + g]) for br, w in enumerate((wqa, wqb))]

    wq_lo = pl.ds(0, SH * 128)
    wq_hi = pl.ds((32 + SH) * 128, (16 - SH) * 128)

    def wq0_copies(br, r):
        out = []
        for rr, cols, sm in ((r - 1, wq_hi, 1), (r, wq_lo, 0)):
            if 0 <= rr < QRT:
                rows = pl.ds(rr * 8, 8)
                out.append(pltpu.make_async_copy((wqa, wqb)[br].at[rows, cols], wqbuf.at[br, rows, cols],
                                                 sems.at[WQSEM + sm]))
        return out

    def out_copy(r0, nr, c0, nc):
        rows, cols = pl.ds(r0, nr), pl.ds(c0, nc)
        return pltpu.make_async_copy(obuf.at[rows, cols], out_hbm.at[rows, cols], sems.at[OSEM])

    lane = lax.broadcasted_iota(jnp.int32, (SQ, 128), 1)

    def rows_of(blk, r0, nr, c0, nc):
        return jnp.concatenate(
            [blk[:, r * SK + c0:r * SK + c0 + nc] for r in range(r0 // 8, (r0 + nr) // 8)], axis=0)

    def qproj(br, n):
        x = xbuf[br, pl.ds(_mo((n & 7) * SQ, SQ), SQ), :]
        wq = wqbuf[br, :, pl.ds(_mo(_pair_of(n >> 3) * PAIR, 128), PAIR)]
        q = jnp.dot(x, wq, preferred_element_type=F32) * QSCALE
        qb = q[:, 128:256]
        qq = jnp.concatenate([q[:, 0:128], jnp.where(lane < 64, qb, 0.0),
                              jnp.where(lane >= 64, qb, 0.0), q[:, 256:384]], axis=1)
        qbuf[n & 1, br] = qq.astype(BF16)

    def oproj(br, n, o):
        rows = pl.ds(_mo((n & 7) * SQ, SQ), SQ)
        tot = acc[rows, br * D:(br + 1) * D] + jnp.dot(
            o, wobuf[(n >> 3) & (NW - 1), br], preferred_element_type=F32)
        acc[rows, br * D:(br + 1) * D] = tot
        obuf[rows, br * D:(br + 1) * D] = tot.astype(BF16)

    def qk(br, n, hook):
        qq = qbuf[n & 1, br]
        kt = kvbuf.at[n & (NBUF - 1), br, 0]
        parts = []
        for h in range(2):
            for c in range(2):
                parts.append(jnp.dot(qq[:, h * 256:(h + 1) * 256], rows_of(kt, h * 128, 256, c * 512, 512),
                                     preferred_element_type=F32))
                hook()
        return jnp.concatenate(parts[0:2], axis=1), jnp.concatenate(parts[2:4], axis=1)

    def softmax_pv(s, br, n, h):
        m = jnp.max(s, axis=-1, keepdims=True)
        p = jnp.exp2(s - m)
        l = jnp.sum(p, axis=-1, keepdims=True)
        vt = rows_of(kvbuf.at[n & (NBUF - 1), br, 1], h * DH, DH, 0, SK)
        ot = lax.dot_general(vt, p.astype(BF16), NT, preferred_element_type=F32)
        return ot, jnp.broadcast_to(1.0 / l, (SQ, 128))

    def mk_inv(i1, i2):
        return jnp.concatenate([i1, jnp.where(lane < 64, i1, i2), i2], axis=1)

    def mk_o(ot1, i1, ot2, i2):
        return (jnp.concatenate([ot1, ot2], axis=0).T * mk_inv(i1, i2)).astype(BF16)

    def carried_o():
        rest = (otbuf[...].T * invbuf[...]).astype(BF16)
        return jnp.concatenate([o0buf[...], rest], axis=1)

    xs = [[pltpu.make_async_copy(src.at[pl.ds(c * 32, 32), :], xbuf.at[br, pl.ds(c * 32, 32), :], sems.at[XSEM])]
          for c in range(B * SQ // 32) for br, src in enumerate((xa, xb))]
    wos = [[c] for g, nj in ((0, B), (1, WLEAD)) for j in range(nj) for h in range(2) for c in wo_copies(g, j, h)]
    wqs = [wq0_copies(br, r) for r in range(QRT + 1) for br in range(2)]
    single, paired = [], []
    for i in range(-5, 0):
        for t in range(NSTEP):
            plan = [e for e in step_plan(i, t) if e[0]]
            if len(plan) == 8:
                paired += plan
            else:
                single += [[kv_copy(*args)] for _, args, _ in plan]
    merged = sorted([((q + 0.5) / len(lst), r, q) for r, lst in enumerate((xs, wos, wqs, single))
                     for q in range(len(lst))])
    for pos, (_, r, q) in enumerate(merged):
        for c in (xs, wos, wqs, single)[r][q]:
            c.start(priority=pos % 2)
    for _, args, prio in paired:
        kv_copy(*args).start(priority=prio)

    acc[...] = jnp.zeros(acc.shape, F32)
    o0buf[...] = jnp.zeros(o0buf.shape, BF16)
    otbuf[...] = jnp.zeros(otbuf.shape, F32)
    invbuf[...] = jnp.zeros(invbuf.shape, F32)

    wait_all(xbuf, XSEM)
    wait_all(wqbuf.at[:, :, wq_lo], WQSEM)
    wait_all(wqbuf.at[:, :, wq_hi], WQSEM + 1)
    wait_all(wobuf.at[0], WOSEM)
    for n in range(2):
        qproj(0, n)
        qproj(1, n)

    def body(i, carry):
        slot = i & (NBUF - 1)
        wait_all(kvbuf.at[slot], KVSEM + slot)

        for g in range(2):
            @pl.when(i == ((SH + 16 * g) // 3 + 1) * B - 2)
            def _(g=g):
                wait_all(wqbuf.at[:, :, wq_cols(g)], WQSEM + 2 + g)

        @pl.when(jnp.logical_and((i & 7) == 0, i > 0))
        def _():
            ws = (i >> 3) & (NW - 1)
            wait_all(wobuf.at[ws], WOSEM + ws)

        step = [0]

        def hook():
            t = step[0]
            step[0] += 1
            for ok, args, prio in step_plan(i, t):
                @pl.when(ok)
                def _(args=args, prio=prio):
                    kv_copy(*args).start(priority=prio)
            if t in WAT:
                gw = ((i + WLEAD) >> 3) + 1

                @pl.when(gw < NHP)
                def _():
                    for q, c in enumerate(wo_copies(gw, (i + WLEAD) & 7, WAT.index(t))):
                        c.start(priority=q)
            if t in QAT:
                @pl.when(jnp.logical_and(i < 64, (i & 1) == 0))
                def _():
                    for q, c in enumerate(wq_copies(i, QAT.index(t))):
                        c.start(priority=q)

        sa1, sa2 = qk(0, i, hook)
        oproj(1, jnp.maximum(i - 1, 0), carried_o())
        ota1, ia1 = softmax_pv(sa1, 0, i, 0)
        hook()
        qproj(0, i + 2)
        ota2, ia2 = softmax_pv(sa2, 0, i, 1)
        hook()
        sb1, sb2 = qk(1, i, hook)
        oproj(0, i, mk_o(ota1, ia1, ota2, ia2))
        otb1, ib1 = softmax_pv(sb1, 1, i, 0)
        hook()
        qproj(1, i + 2)
        otb2, ib2 = softmax_pv(sb2, 1, i, 1)
        hook()
        o0buf[...] = (otb1[0:128, :].T * ib1).astype(BF16)
        otbuf[0:DH - 128, :] = otb1[128:DH, :]
        otbuf[DH - 128:PAIR - 128, :] = otb2
        invbuf[...] = mk_inv(ib1, ib2)[:, 128:PAIR]
        assert step[0] == NSTEP
        return carry

    lax.fori_loop(0, NI - 2, body, 0)

    for i in (NI - 2, NI - 1):
        wait_all(kvbuf.at[i & (NBUF - 1)], KVSEM + (i & (NBUF - 1)))
        if i == NI - 1:
            for c in range(SQ // OCH):
                for b in range(B - 1):
                    out_copy(b * SQ + c * OCH, OCH, 0, 2 * D).start(priority=(c + b) % 2)
        tail_step = [0]

        def tail_hook():
            for ok, args, prio in step_plan(i, tail_step[0]):
                if ok:
                    kv_copy(*args).start(priority=prio)
            tail_step[0] += 1

        sa1, sa2 = qk(0, i, tail_hook)
        if i == NI - 2:
            oproj(1, i - 1, carried_o())
            ota1, ia1 = softmax_pv(sa1, 0, i, 0)
            tail_hook()
            sb1, sb2 = qk(1, i, tail_hook)
        else:
            sb1, sb2 = qk(1, i, tail_hook)
            ota1, ia1 = softmax_pv(sa1, 0, i, 0)
            tail_hook()
        ota2, ia2 = softmax_pv(sa2, 0, i, 1)
        tail_hook()
        otb1, ib1 = softmax_pv(sb1, 1, i, 0)
        tail_hook()
        otb2, ib2 = softmax_pv(sb2, 1, i, 1)
        tail_hook()
        assert tail_step[0] == NSTEP
        oproj(0, i, mk_o(ota1, ia1, ota2, ia2))
        if i == NI - 1:
            out_copy((B - 1) * SQ, SQ, 0, D).start()
        oproj(1, i, mk_o(otb1, ib1, otb2, ib2))
    out_copy((B - 1) * SQ, SQ, D, D).start()
    out_copy(0, B * SQ, 0, 2 * D).wait()


@jax.jit
def pallas_concat_heads__mha_block_cached__gqa_block_cached__near_ridge_kernel(
    A_x, A_k_cache, A_v_cache, A_wq, A_wo, B_x, B_k_cache, B_v_cache, B_wq, B_wo,
):
    def kv(a):
        a = jnp.swapaxes(a, 2, 3).reshape(B, NHP, PAIR // 8, 8, SK)
        return jnp.swapaxes(a, 2, 3).reshape(B, NHP, 8, WIDE)

    any_spec = pl.BlockSpec(memory_space=pl.ANY)
    out = pl.pallas_call(
        _kernel,
        in_specs=[any_spec] * 10,
        out_specs=any_spec,
        out_shape=jax.ShapeDtypeStruct((B * SQ, 2 * D), BF16),
        scratch_shapes=[
            pltpu.VMEM((NBUF, 2, 2, 8, WIDE), BF16),
            pltpu.VMEM((2, D, H * DH), BF16),
            pltpu.VMEM((NW, 2, PAIR, D), BF16),
            pltpu.VMEM((2, B * SQ, D), BF16),
            pltpu.VMEM((B * SQ, 2 * D), F32),
            pltpu.VMEM((B * SQ, 2 * D), BF16),
            pltpu.VMEM((2, 2, SQ, 512), BF16),
            pltpu.VMEM((SQ, 128), BF16),
            pltpu.VMEM((PAIR - 128, SQ), F32),
            pltpu.VMEM((SQ, PAIR - 128), F32),
            pltpu.SemaphoreType.DMA((NSEM,)),
        ],
        compiler_params=pltpu.CompilerParams(
            vmem_limit_bytes=100 * 1024 * 1024,
        ),
    )(A_x.reshape(B * SQ, D), kv(A_k_cache), kv(A_v_cache), A_wq, A_wo,
      B_x.reshape(B * SQ, D), kv(B_k_cache), kv(B_v_cache), B_wq, B_wo)
    return out.reshape(B, SQ, 2 * D)
```

```python
import math
import jax
import jax.numpy as jnp
from jax import lax
import jax.experimental.pallas as pl
import jax.experimental.pallas.tpu as pltpu

B, SQ, D = 8, 128, 640
H, SK, DH = 32, 1024, 192
PAIR = 2 * DH
NHP = H // 2
NI = NHP * B
QSCALE = (DH ** -0.5) * math.log2(math.e)
NBUF = 8
NW = 4
NSTEP = 12
PH = 6
I0 = 110
ROT = 3
ALLOC = (2, 2, 1, 1)
WAT = (0, 6)
QAT = (1, 3, 5, 7, 9)
WLEAD = 2
OCH = 16
SH = 13
F32 = jnp.float32
BF16 = jnp.bfloat16
NT = (((1,), (1,)), ((), ()))

assert 12 <= SH <= 13
QRT = D // 8
NTILE = (PAIR // 8) * (SK // 128)
WIDE = NTILE * 128
_CUTS = [0] + [SH + 16 * k for k in range(NTILE // 16 - 1)] + [NTILE]
VISITS = list(zip(_CUTS[:-1], _CUTS[1:]))
KVSEM, WOSEM, WQSEM, XSEM, OSEM = 0, NBUF, NBUF + NW, NBUF + NW + 4, NBUF + NW + 5
NSEM = OSEM + 1


def _mo(x, m):
    return x if isinstance(x, int) else pl.multiple_of(x, m)


def _pair_of(g):
    return (g + (NHP - 1)) & (NHP - 1)


def _kernel(xa, ka, va, wqa, woa, xb, kb, vb, wqb, wob, out_hbm,
            kvbuf, wqbuf, wobuf, xbuf, acc, obuf, qbuf, o0buf, otbuf, invbuf, sems):

    def wait_all(ref, sem):
        pltpu.make_async_copy(ref, ref, sems.at[sem]).wait()

    def kv_copy(n, br, kv, k):
        t0, t1 = VISITS[k]
        cols = pl.ds(t0 * 128, (t1 - t0) * 128)
        slot = n & (NBUF - 1)
        src = ((ka, va), (kb, vb))[br][kv]
        return pltpu.make_async_copy(src.at[n & 7, _pair_of(n >> 3), :, cols],
                                     kvbuf.at[slot, br, kv, :, cols], sems.at[KVSEM + slot])

    def step_plan(i, t):
        vi = i + (t + PH) // NSTEP
        m, br = divmod((t + PH) % NSTEP, 2)
        n1 = vi + 1
        if isinstance(vi, int):
            n0 = vi + 2 + (1 if vi < I0 else 0)
            ok1, ok0 = 0 <= n1 < NI, 0 <= n0 < NI and vi != I0
        else:
            n0 = vi + 2 + (vi < I0).astype(jnp.int32)
            ok1, ok0 = n1 < NI, jnp.logical_and(n0 < NI, vi != I0)
        late = [(n1, br, kv, 11 + 2 * ((m + ROT) % 6) + h) for kv in range(2) for h in range(2)]
        if m == 0:
            early = [(n0, b2, kv, (0, 23)[br]) for b2 in range(2) for kv in range(2)]
        else:
            early = [(n0, br, kv, 2 * m - 1 + h) for kv in range(2) for h in range(2)]
        plan = []
        for a1, a0 in zip(late, early):
            plan.append((ok1, a1, 0))
            plan.append((ok0, a0, 1))
        return plan

    def wo_copies(g, j, h):
        slot = g & (NW - 1)
        r0 = _mo(j * 48 + h * 24, 8)
        return [pltpu.make_async_copy(w.at[pl.ds(_mo(_pair_of(g) * PAIR + r0, 8), 24), :],
                                      wobuf.at[slot, br, pl.ds(r0, 24), :], sems.at[WOSEM + slot])
                for br, w in enumerate((woa, wob))]

    def wq_cols(g):
        return pl.ds(_mo((SH + 16 * g) * 128, 128), 2048)

    def wq_copies(i, k):
        g = (i >> 5) & 1
        rows = pl.ds(pl.multiple_of((((i >> 1) & 15) * 5 + k) * 8, 8), 8)
        return [pltpu.make_async_copy(w.at[rows, wq_cols(g)], wqbuf.at[br, rows, wq_cols(g)],
                                      sems.at[WQSEM + 2 + g]) for br, w in enumerate((wqa, wqb))]

    wq_lo = pl.ds(0, SH * 128)
    wq_hi = pl.ds((32 + SH) * 128, (16 - SH) * 128)

    def wq0_copies(br, r):
        out = []
        for rr, cols, sm in ((r - 1, wq_hi, 1), (r, wq_lo, 0)):
            if 0 <= rr < QRT:
                rows = pl.ds(rr * 8, 8)
                out.append(pltpu.make_async_copy((wqa, wqb)[br].at[rows, cols], wqbuf.at[br, rows, cols],
                                                 sems.at[WQSEM + sm]))
        return out

    def out_copy(r0, nr, c0, nc):
        rows, cols = pl.ds(r0, nr), pl.ds(c0, nc)
        return pltpu.make_async_copy(obuf.at[rows, cols], out_hbm.at[rows, cols], sems.at[OSEM])

    lane = lax.broadcasted_iota(jnp.int32, (SQ, 128), 1)

    def rows_of(blk, r0, nr):
        v = blk[:, (r0 // 8) * SK:((r0 + nr) // 8) * SK]
        return jnp.concatenate([v[:, r * SK:(r + 1) * SK] for r in range(nr // 8)], axis=0)

    def qproj(br, n):
        x = xbuf[br, pl.ds(_mo((n & 7) * SQ, SQ), SQ), :]
        wq = wqbuf[br, :, pl.ds(_mo(_pair_of(n >> 3) * PAIR, 128), PAIR)]
        q = jnp.dot(x, wq, preferred_element_type=F32) * QSCALE
        qb = q[:, 128:256]
        qq = jnp.concatenate([q[:, 0:128], jnp.where(lane < 64, qb, 0.0),
                              jnp.where(lane >= 64, qb, 0.0), q[:, 256:384]], axis=1)
        qbuf[n & 1, br] = qq.astype(BF16)

    def oproj(br, n, o):
        rows = pl.ds(_mo((n & 7) * SQ, SQ), SQ)
        tot = acc[rows, br * D:(br + 1) * D] + jnp.dot(
            o, wobuf[(n >> 3) & (NW - 1), br], preferred_element_type=F32)
        acc[rows, br * D:(br + 1) * D] = tot
        obuf[rows, br * D:(br + 1) * D] = tot.astype(BF16)

    def qk(br, n, hook):
        qq = qbuf[n & 1, br]
        kt = kvbuf.at[n & (NBUF - 1), br, 0]
        s = []
        for h in range(2):
            s.append(jnp.dot(qq[:, h * 256:(h + 1) * 256], rows_of(kt, h * 128, 256), preferred_element_type=F32))
            hook(ALLOC[h])
        return s

    def softmax_pv(s, br, n, h):
        m = jnp.max(s, axis=-1, keepdims=True)
        p = jnp.exp2(s - m)
        l = jnp.sum(p, axis=-1, keepdims=True)
        vt = rows_of(kvbuf.at[n & (NBUF - 1), br, 1], h * DH, DH)
        ot = lax.dot_general(vt, p.astype(BF16), NT, preferred_element_type=F32)
        return ot, jnp.broadcast_to(1.0 / l, (SQ, 128))

    def mk_inv(i1, i2):
        return jnp.concatenate([i1, jnp.where(lane < 64, i1, i2), i2], axis=1)

    def mk_o(ot1, i1, ot2, i2):
        return (jnp.concatenate([ot1, ot2], axis=0).T * mk_inv(i1, i2)).astype(BF16)

    def carried_o():
        rest = (otbuf[...].T * invbuf[...]).astype(BF16)
        return jnp.concatenate([o0buf[...], rest], axis=1)

    xs = [[pltpu.make_async_copy(src.at[pl.ds(c * 32, 32), :], xbuf.at[br, pl.ds(c * 32, 32), :], sems.at[XSEM])]
          for c in range(B * SQ // 32) for br, src in enumerate((xa, xb))]
    wos = [[c] for g, nj in ((0, B), (1, WLEAD)) for j in range(nj) for h in range(2) for c in wo_copies(g, j, h)]
    wqs = [wq0_copies(br, r) for r in range(QRT + 1) for br in range(2)]
    single, paired = [], []
    for i in range(-5, 0):
        for t in range(NSTEP):
            plan = [e for e in step_plan(i, t) if e[0]]
            if len(plan) == 8:
                paired += plan
            else:
                single += [[kv_copy(*args)] for _, args, _ in plan]
    merged = sorted([((q + 0.5) / len(lst), r, q) for r, lst in enumerate((xs, wos, wqs, single))
                     for q in range(len(lst))])
    for pos, (_, r, q) in enumerate(merged):
        for c in (xs, wos, wqs, single)[r][q]:
            c.start(priority=pos % 2)
    for _, args, prio in paired:
        kv_copy(*args).start(priority=prio)

    acc[...] = jnp.zeros(acc.shape, F32)
    o0buf[...] = jnp.zeros(o0buf.shape, BF16)
    otbuf[...] = jnp.zeros(otbuf.shape, F32)
    invbuf[...] = jnp.zeros(invbuf.shape, F32)

    wait_all(xbuf, XSEM)
    wait_all(wqbuf.at[:, :, wq_lo], WQSEM)
    wait_all(wqbuf.at[:, :, wq_hi], WQSEM + 1)
    wait_all(wobuf.at[0], WOSEM)
    for n in range(2):
        qproj(0, n)
        qproj(1, n)

    def body(i, carry):
        slot = i & (NBUF - 1)
        wait_all(kvbuf.at[slot], KVSEM + slot)

        for g in range(2):
            @pl.when(i == ((SH + 16 * g) // 3 + 1) * B - 2)
            def _(g=g):
                wait_all(wqbuf.at[:, :, wq_cols(g)], WQSEM + 2 + g)

        @pl.when(jnp.logical_and((i & 7) == 0, i > 0))
        def _():
            ws = (i >> 3) & (NW - 1)
            wait_all(wobuf.at[ws], WOSEM + ws)

        step = [0]

        def hook(count):
            for _ in range(count):
                one_step()

        def one_step():
            t = step[0]
            step[0] += 1
            for ok, args, prio in step_plan(i, t):
                @pl.when(ok)
                def _(args=args, prio=prio):
                    kv_copy(*args).start(priority=prio)
            if t in WAT:
                gw = ((i + WLEAD) >> 3) + 1

                @pl.when(gw < NHP)
                def _():
                    for q, c in enumerate(wo_copies(gw, (i + WLEAD) & 7, WAT.index(t))):
                        c.start(priority=q)
            if t in QAT:
                @pl.when(jnp.logical_and(i < 64, (i & 1) == 0))
                def _():
                    for q, c in enumerate(wq_copies(i, QAT.index(t))):
                        c.start(priority=q)

        sa1, sa2 = qk(0, i, hook)
        oproj(1, jnp.maximum(i - 1, 0), carried_o())
        ota1, ia1 = softmax_pv(sa1, 0, i, 0)
        hook(ALLOC[2])
        qproj(0, i + 2)
        ota2, ia2 = softmax_pv(sa2, 0, i, 1)
        hook(ALLOC[3])
        sb1, sb2 = qk(1, i, hook)
        oproj(0, i, mk_o(ota1, ia1, ota2, ia2))
        otb1, ib1 = softmax_pv(sb1, 1, i, 0)
        hook(ALLOC[2])
        qproj(1, i + 2)
        otb2, ib2 = softmax_pv(sb2, 1, i, 1)
        hook(ALLOC[3])
        o0buf[...] = (otb1[0:128, :].T * ib1).astype(BF16)
        otbuf[0:DH - 128, :] = otb1[128:DH, :]
        otbuf[DH - 128:PAIR - 128, :] = otb2
        invbuf[...] = mk_inv(ib1, ib2)[:, 128:PAIR]
        assert step[0] == NSTEP
        return carry

    lax.fori_loop(0, NI - 2, body, 0)

    for i in (NI - 2, NI - 1):
        wait_all(kvbuf.at[i & (NBUF - 1)], KVSEM + (i & (NBUF - 1)))
        if i == NI - 1:
            for c in range(SQ // OCH):
                for b in range(B - 1):
                    out_copy(b * SQ + c * OCH, OCH, 0, 2 * D).start(priority=(c + b) % 2)
        tail_step = [0]

        def tail_hook(count):
            for _ in range(count):
                for ok, args, prio in step_plan(i, tail_step[0]):
                    if ok:
                        kv_copy(*args).start(priority=prio)
                tail_step[0] += 1

        sa1, sa2 = qk(0, i, tail_hook)
        if i == NI - 2:
            oproj(1, i - 1, carried_o())
            ota1, ia1 = softmax_pv(sa1, 0, i, 0)
            tail_hook(ALLOC[2])
            sb1, sb2 = qk(1, i, tail_hook)
        else:
            sb1, sb2 = qk(1, i, tail_hook)
            ota1, ia1 = softmax_pv(sa1, 0, i, 0)
            tail_hook(ALLOC[2])
        ota2, ia2 = softmax_pv(sa2, 0, i, 1)
        tail_hook(ALLOC[3])
        otb1, ib1 = softmax_pv(sb1, 1, i, 0)
        tail_hook(ALLOC[2])
        otb2, ib2 = softmax_pv(sb2, 1, i, 1)
        tail_hook(ALLOC[3])
        assert tail_step[0] == NSTEP
        oproj(0, i, mk_o(ota1, ia1, ota2, ia2))
        if i == NI - 1:
            out_copy((B - 1) * SQ, SQ, 0, D).start()
        oproj(1, i, mk_o(otb1, ib1, otb2, ib2))
    out_copy((B - 1) * SQ, SQ, D, D).start()
    out_copy(0, B * SQ, 0, 2 * D).wait()


@jax.jit
def pallas_concat_heads__mha_block_cached__gqa_block_cached__near_ridge_kernel(
    A_x, A_k_cache, A_v_cache, A_wq, A_wo, B_x, B_k_cache, B_v_cache, B_wq, B_wo,
):
    def kv(a):
        a = jnp.swapaxes(a, 2, 3).reshape(B, NHP, PAIR // 8, 8, SK)
        return jnp.swapaxes(a, 2, 3).reshape(B, NHP, 8, WIDE)

    any_spec = pl.BlockSpec(memory_space=pl.ANY)
    out = pl.pallas_call(
        _kernel,
        in_specs=[any_spec] * 10,
        out_specs=any_spec,
        out_shape=jax.ShapeDtypeStruct((B * SQ, 2 * D), BF16),
        scratch_shapes=[
            pltpu.VMEM((NBUF, 2, 2, 8, WIDE), BF16),
            pltpu.VMEM((2, D, H * DH), BF16),
            pltpu.VMEM((NW, 2, PAIR, D), BF16),
            pltpu.VMEM((2, B * SQ, D), BF16),
            pltpu.VMEM((B * SQ, 2 * D), F32),
            pltpu.VMEM((B * SQ, 2 * D), BF16),
            pltpu.VMEM((2, 2, SQ, 512), BF16),
            pltpu.VMEM((SQ, 128), BF16),
            pltpu.VMEM((PAIR - 128, SQ), F32),
            pltpu.VMEM((SQ, PAIR - 128), F32),
            pltpu.SemaphoreType.DMA((NSEM,)),
        ],
        compiler_params=pltpu.CompilerParams(
            vmem_limit_bytes=100 * 1024 * 1024,
        ),
    )(A_x.reshape(B * SQ, D), kv(A_k_cache), kv(A_v_cache), A_wq, A_wo,
      B_x.reshape(B * SQ, D), kv(B_k_cache), kv(B_v_cache), B_wq, B_wo)
    return out.reshape(B, SQ, 2 * D)
```

```python
import math
import jax
import jax.numpy as jnp
from jax import lax
import jax.experimental.pallas as pl
import jax.experimental.pallas.tpu as pltpu

B, SQ, D = 8, 128, 640
H, SK, DH = 32, 1024, 192
PAIR = 2 * DH
NHP = H // 2
NI = NHP * B
QSCALE = (DH ** -0.5) * math.log2(math.e)
NBUF = 8
NW = 4
NSTEP = 12
PH = 6
I0 = 108
ROT = 3
ALLOC = (2, 2, 1, 1)
WAT = (0, 6)
QAT = (1, 3, 5, 7, 9)
WLEAD = 2
OCH = 16
SH = 13
F32 = jnp.float32
BF16 = jnp.bfloat16
NT = (((1,), (1,)), ((), ()))

assert PH <= NSTEP
assert 12 <= SH <= 13
QRT = D // 8
NTILE = (PAIR // 8) * (SK // 128)
WIDE = NTILE * 128
_CUTS = [0] + [SH + 16 * k for k in range(NTILE // 16 - 1)] + [NTILE]
VISITS = list(zip(_CUTS[:-1], _CUTS[1:]))
KVSEM, WOSEM, WQSEM, XSEM, OSEM = 0, NBUF, NBUF + NW, NBUF + NW + 4, NBUF + NW + 5
NSEM = OSEM + 1


def _mo(x, m):
    return x if isinstance(x, int) else pl.multiple_of(x, m)


def _pair_of(g):
    return (g + (NHP - 1)) & (NHP - 1)


def _kernel(xa, ka, va, wqa, woa, xb, kb, vb, wqb, wob, out_hbm,
            kvbuf, wqbuf, wobuf, xbuf, acc, obuf, qbuf, o0buf, otbuf, invbuf, sems):

    def wait_all(ref, sem):
        pltpu.make_async_copy(ref, ref, sems.at[sem]).wait()

    def kv_copy(n, br, kv, k):
        t0, t1 = VISITS[k]
        cols = pl.ds(t0 * 128, (t1 - t0) * 128)
        slot = n & (NBUF - 1)
        src = ((ka, va), (kb, vb))[br][kv]
        return pltpu.make_async_copy(src.at[n & 7, _pair_of(n >> 3), :, cols],
                                     kvbuf.at[slot, br, kv, :, cols], sems.at[KVSEM + slot])

    def step_plan(i, t):
        vi = i + (t + PH) // NSTEP
        m, br = divmod((t + PH) % NSTEP, 2)
        n1 = vi + 1
        if isinstance(vi, int):
            n0 = vi + 2 + (1 if vi < I0 else 0)
            ok1, ok0 = 0 <= n1 < NI, 0 <= n0 < NI and vi != I0
        else:
            n0 = vi + 2 + (vi < I0).astype(jnp.int32)
            ok1, ok0 = True, jnp.logical_and(n0 < NI, vi != I0)
        late = [(n1, br, kv, 11 + 2 * ((m + ROT) % 6) + h) for kv in range(2) for h in range(2)]
        if m == 0:
            early = [(n0, b2, kv, (0, 23)[br]) for b2 in range(2) for kv in range(2)]
        else:
            early = [(n0, br, kv, 2 * m - 1 + h) for kv in range(2) for h in range(2)]
        plan = []
        for a1, a0 in zip(late, early):
            plan.append((ok1, a1, 0))
            plan.append((ok0, a0, 1))
        return plan

    def wo_copies(g, j, h):
        slot = g & (NW - 1)
        r0 = _mo(j * 48 + h * 24, 8)
        return [pltpu.make_async_copy(w.at[pl.ds(_mo(_pair_of(g) * PAIR + r0, 8), 24), :],
                                      wobuf.at[slot, br, pl.ds(r0, 24), :], sems.at[WOSEM + slot])
                for br, w in enumerate((woa, wob))]

    def wq_cols(g):
        return pl.ds(_mo((SH + 16 * g) * 128, 128), 2048)

    def wq_copies(i, k):
        g = (i >> 5) & 1
        rows = pl.ds(pl.multiple_of((((i >> 1) & 15) * 5 + k) * 8, 8), 8)
        return [pltpu.make_async_copy(w.at[rows, wq_cols(g)], wqbuf.at[br, rows, wq_cols(g)],
                                      sems.at[WQSEM + 2 + g]) for br, w in enumerate((wqa, wqb))]

    wq_lo = pl.ds(0, SH * 128)
    wq_hi = pl.ds((32 + SH) * 128, (16 - SH) * 128)

    def wq0_copies(br, r):
        out = []
        for rr, cols, sm in ((r - 1, wq_hi, 1), (r, wq_lo, 0)):
            if 0 <= rr < QRT:
                rows = pl.ds(rr * 8, 8)
                out.append(pltpu.make_async_copy((wqa, wqb)[br].at[rows, cols], wqbuf.at[br, rows, cols],
                                                 sems.at[WQSEM + sm]))
        return out

    def out_copy(r0, nr, c0, nc):
        rows, cols = pl.ds(r0, nr), pl.ds(c0, nc)
        return pltpu.make_async_copy(obuf.at[rows, cols], out_hbm.at[rows, cols], sems.at[OSEM])

    lane = lax.broadcasted_iota(jnp.int32, (SQ, 128), 1)

    def rows_of(blk, r0, nr):
        v = blk[:, (r0 // 8) * SK:((r0 + nr) // 8) * SK]
        return jnp.concatenate([v[:, r * SK:(r + 1) * SK] for r in range(nr // 8)], axis=0)

    def qproj(br, n):
        x = xbuf[br, pl.ds(_mo((n & 7) * SQ, SQ), SQ), :]
        wq = wqbuf[br, :, pl.ds(_mo(_pair_of(n >> 3) * PAIR, 128), PAIR)]
        q = jnp.dot(x, wq, preferred_element_type=F32) * QSCALE
        qb = q[:, 128:256]
        qq = jnp.concatenate([q[:, 0:128], jnp.where(lane < 64, qb, 0.0),
                              jnp.where(lane >= 64, qb, 0.0), q[:, 256:384]], axis=1)
        qbuf[n & 1, br] = qq.astype(BF16)

    def oproj(br, n, o):
        rows = pl.ds(_mo((n & 7) * SQ, SQ), SQ)
        tot = acc[rows, br * D:(br + 1) * D] + jnp.dot(
            o, wobuf[(n >> 3) & (NW - 1), br], preferred_element_type=F32)
        acc[rows, br * D:(br + 1) * D] = tot
        obuf[rows, br * D:(br + 1) * D] = tot.astype(BF16)

    def qk(br, n, hook):
        qq = qbuf[n & 1, br]
        kt = kvbuf.at[n & (NBUF - 1), br, 0]
        s = []
        for h in range(2):
            s.append(jnp.dot(qq[:, h * 256:(h + 1) * 256], rows_of(kt, h * 128, 256), preferred_element_type=F32))
            hook(ALLOC[h])
        return s

    def softmax_pv(s, br, n, h):
        m = jnp.max(s, axis=-1, keepdims=True)
        p = jnp.exp2(s - m)
        l = jnp.sum(p, axis=-1, keepdims=True)
        vt = rows_of(kvbuf.at[n & (NBUF - 1), br, 1], h * DH, DH)
        ot = lax.dot_general(vt, p.astype(BF16), NT, preferred_element_type=F32)
        return ot, jnp.broadcast_to(1.0 / l, (SQ, 128))

    def mk_inv(i1, i2):
        return jnp.concatenate([i1, jnp.where(lane < 64, i1, i2), i2], axis=1)

    def mk_o(ot1, i1, ot2, i2):
        return (jnp.concatenate([ot1, ot2], axis=0).T * mk_inv(i1, i2)).astype(BF16)

    def carried_o():
        rest = (otbuf[...].T * invbuf[...]).astype(BF16)
        return jnp.concatenate([o0buf[...], rest], axis=1)

    xs = [[pltpu.make_async_copy(src.at[pl.ds(c * 32, 32), :], xbuf.at[br, pl.ds(c * 32, 32), :], sems.at[XSEM])]
          for c in range(B * SQ // 32) for br, src in enumerate((xa, xb))]
    wos = [[c] for g, nj in ((0, B), (1, WLEAD)) for j in range(nj) for h in range(2) for c in wo_copies(g, j, h)]
    wqs = [wq0_copies(br, r) for r in range(QRT + 1) for br in range(2)]
    single, paired = [], []
    for i in range(-5, 0):
        for t in range(NSTEP):
            plan = [e for e in step_plan(i, t) if e[0]]
            if len(plan) == 8:
                paired += plan
            else:
                single += [[kv_copy(*args)] for _, args, _ in plan]
    merged = sorted([((q + 0.5) / len(lst), r, q) for r, lst in enumerate((xs, wos, wqs, single))
                     for q in range(len(lst))])
    for pos, (_, r, q) in enumerate(merged):
        for c in (xs, wos, wqs, single)[r][q]:
            c.start(priority=pos % 2)
    for _, args, prio in paired:
        kv_copy(*args).start(priority=prio)

    acc[...] = jnp.zeros(acc.shape, F32)
    o0buf[...] = jnp.zeros(o0buf.shape, BF16)
    otbuf[...] = jnp.zeros(otbuf.shape, F32)
    invbuf[...] = jnp.zeros(invbuf.shape, F32)

    wait_all(xbuf, XSEM)
    wait_all(wqbuf.at[:, :, wq_lo], WQSEM)
    wait_all(wqbuf.at[:, :, wq_hi], WQSEM + 1)
    wait_all(wobuf.at[0], WOSEM)
    for n in range(2):
        qproj(0, n)
        qproj(1, n)

    def body(i, carry):
        slot = i & (NBUF - 1)
        wait_all(kvbuf.at[slot], KVSEM + slot)

        for g in range(2):
            @pl.when(i == ((SH + 16 * g) // 3 + 1) * B - 2)
            def _(g=g):
                wait_all(wqbuf.at[:, :, wq_cols(g)], WQSEM + 2 + g)

        @pl.when(jnp.logical_and((i & 7) == 0, i > 0))
        def _():
            ws = (i >> 3) & (NW - 1)
            wait_all(wobuf.at[ws], WOSEM + ws)

        step = [0]

        def hook(count):
            for _ in range(count):
                one_step()

        def one_step():
            t = step[0]
            step[0] += 1
            for ok, args, prio in step_plan(i, t):
                def start(args=args, prio=prio):
                    kv_copy(*args).start(priority=prio)
                if ok is True:
                    start()
                else:
                    pl.when(ok)(start)
            if t in WAT:
                gw = ((i + WLEAD) >> 3) + 1

                @pl.when(gw < NHP)
                def _():
                    for q, c in enumerate(wo_copies(gw, (i + WLEAD) & 7, WAT.index(t))):
                        c.start(priority=q)
            if t in QAT:
                @pl.when(jnp.logical_and(i < 64, (i & 1) == 0))
                def _():
                    for q, c in enumerate(wq_copies(i, QAT.index(t))):
                        c.start(priority=q)

        sa1, sa2 = qk(0, i, hook)
        oproj(1, jnp.maximum(i - 1, 0), carried_o())
        ota1, ia1 = softmax_pv(sa1, 0, i, 0)
        hook(ALLOC[2])
        qproj(0, i + 2)
        ota2, ia2 = softmax_pv(sa2, 0, i, 1)
        hook(ALLOC[3])
        sb1, sb2 = qk(1, i, hook)
        oproj(0, i, mk_o(ota1, ia1, ota2, ia2))
        otb1, ib1 = softmax_pv(sb1, 1, i, 0)
        hook(ALLOC[2])
        qproj(1, i + 2)
        otb2, ib2 = softmax_pv(sb2, 1, i, 1)
        hook(ALLOC[3])
        o0buf[...] = (otb1[0:128, :].T * ib1).astype(BF16)
        otbuf[0:DH - 128, :] = otb1[128:DH, :]
        otbuf[DH - 128:PAIR - 128, :] = otb2
        invbuf[...] = mk_inv(ib1, ib2)[:, 128:PAIR]
        assert step[0] == NSTEP
        return carry

    lax.fori_loop(0, NI - 2, body, 0)

    for i in (NI - 2, NI - 1):
        wait_all(kvbuf.at[i & (NBUF - 1)], KVSEM + (i & (NBUF - 1)))
        if i == NI - 1:
            for c in range(SQ // OCH):
                for b in range(B - 1):
                    out_copy(b * SQ + c * OCH, OCH, 0, 2 * D).start(priority=(c + b) % 2)
        tail_step = [0]

        def tail_hook(count):
            for _ in range(count):
                for ok, args, prio in step_plan(i, tail_step[0]):
                    if ok:
                        kv_copy(*args).start(priority=prio)
                tail_step[0] += 1

        sa1, sa2 = qk(0, i, tail_hook)
        if i == NI - 2:
            oproj(1, i - 1, carried_o())
            ota1, ia1 = softmax_pv(sa1, 0, i, 0)
            tail_hook(ALLOC[2])
            sb1, sb2 = qk(1, i, tail_hook)
        else:
            sb1, sb2 = qk(1, i, tail_hook)
            ota1, ia1 = softmax_pv(sa1, 0, i, 0)
            tail_hook(ALLOC[2])
        ota2, ia2 = softmax_pv(sa2, 0, i, 1)
        tail_hook(ALLOC[3])
        otb1, ib1 = softmax_pv(sb1, 1, i, 0)
        tail_hook(ALLOC[2])
        otb2, ib2 = softmax_pv(sb2, 1, i, 1)
        tail_hook(ALLOC[3])
        assert tail_step[0] == NSTEP
        oproj(0, i, mk_o(ota1, ia1, ota2, ia2))
        if i == NI - 1:
            out_copy((B - 1) * SQ, SQ, 0, D).start()
        oproj(1, i, mk_o(otb1, ib1, otb2, ib2))
    out_copy((B - 1) * SQ, SQ, D, D).start()
    out_copy(0, B * SQ, 0, 2 * D).wait()


@jax.jit
def pallas_concat_heads__mha_block_cached__gqa_block_cached__near_ridge_kernel(
    A_x, A_k_cache, A_v_cache, A_wq, A_wo, B_x, B_k_cache, B_v_cache, B_wq, B_wo,
):
    def kv(a):
        a = jnp.swapaxes(a, 2, 3).reshape(B, NHP, PAIR // 8, 8, SK)
        return jnp.swapaxes(a, 2, 3).reshape(B, NHP, 8, WIDE)

    any_spec = pl.BlockSpec(memory_space=pl.ANY)
    out = pl.pallas_call(
        _kernel,
        in_specs=[any_spec] * 10,
        out_specs=any_spec,
        out_shape=jax.ShapeDtypeStruct((B * SQ, 2 * D), BF16),
        scratch_shapes=[
            pltpu.VMEM((NBUF, 2, 2, 8, WIDE), BF16),
            pltpu.VMEM((2, D, H * DH), BF16),
            pltpu.VMEM((NW, 2, PAIR, D), BF16),
            pltpu.VMEM((2, B * SQ, D), BF16),
            pltpu.VMEM((B * SQ, 2 * D), F32),
            pltpu.VMEM((B * SQ, 2 * D), BF16),
            pltpu.VMEM((2, 2, SQ, 512), BF16),
            pltpu.VMEM((SQ, 128), BF16),
            pltpu.VMEM((PAIR - 128, SQ), F32),
            pltpu.VMEM((SQ, PAIR - 128), F32),
            pltpu.SemaphoreType.DMA((NSEM,)),
        ],
        compiler_params=pltpu.CompilerParams(
            vmem_limit_bytes=100 * 1024 * 1024,
        ),
    )(A_x.reshape(B * SQ, D), kv(A_k_cache), kv(A_v_cache), A_wq, A_wo,
      B_x.reshape(B * SQ, D), kv(B_k_cache), kv(B_v_cache), B_wq, B_wo)
    return out.reshape(B, SQ, 2 * D)
```
